```python
import jax
import jax.numpy as jnp

def _softmax(x, axis=-1):
    return jax.nn.softmax(x, axis=axis)

def _gelu(x):
    return jax.nn.gelu(x, approximate=True)

def _silu(x):
    return jax.nn.silu(x)

def _sigmoid(x):
    return jax.nn.sigmoid(x)

def _layernorm(x, axis=-1, eps=1e-05):
    m = jnp.mean(x, axis=axis, keepdims=True)
    v = jnp.var(x, axis=axis, keepdims=True)
    return (x - m) / jnp.sqrt(v + eps)

def _scatter_add(tgt, idx, src, axis=0):
    return tgt.at[idx].add(src)

def _segment_sum(src, seg, n):
    return jax.ops.segment_sum(src, seg, n)

class _Rng:

    def __init__(self, key):
        self._k = key

    def _next(self):
        self._k, sub = jax.random.split(self._k)
        return sub

    def normal(self, shape):
        return jax.random.normal(self._next(), shape, dtype=jnp.bfloat16)

    def randint(self, lo, hi, shape):
        return jax.random.randint(self._next(), shape, lo, hi, dtype=jnp.int32)

    def uniform(self, shape, lo=0.0, hi=1.0):
        return jax.random.uniform(self._next(), shape, jnp.bfloat16, lo, hi)

    def permutation(self, n):
        return jax.random.permutation(self._next(), n)
kernel_name = 'adaLN_cond__grouped_kv_mqa__dense_activation_silu__prompt'

def _fwd_setup_inputs():
    _rng = _Rng(jax.random.key(int.from_bytes(__import__("os").urandom(4), "little")))
    _w = lambda a: (lambda t: t.astype(jnp.bfloat16) if jnp.issubdtype(t.dtype, jnp.floating) else t)(jnp.asarray(a))

    def _A_setup():
        B, S, D, H = (1, 2048, 640, 32)
        Dh = D // H
        return {'x': _w((lambda *s: _rng.normal(s) * 0.05)(B, S, D)), 'wq': _w((lambda *s: _rng.normal(s) * 0.05)(D, H * Dh)), 'wk': _w((lambda *s: _rng.normal(s) * 0.05)(D, Dh)), 'wv': _w((lambda *s: _rng.normal(s) * 0.05)(D, Dh)), 'wo': _w((lambda *s: _rng.normal(s) * 0.05)(H * Dh, D))}
    _A_in = _A_setup()

    def _B_setup():
        B, S, D, F = (1, 2048, 640, 1728)
        return {'x': _w((lambda *s: _rng.normal(s) * 0.05)(B, S, D)), 'w1': _w((lambda *s: _rng.normal(s) * 0.05)(D, F) * D ** (-0.5)), 'w2': _w((lambda *s: _rng.normal(s) * 0.05)(F, D) * F ** (-0.5))}
    _B_in = _B_setup()
    return {'A_x': _A_in['x'], 'A_wq': _A_in['wq'], 'A_wk': _A_in['wk'], 'A_wv': _A_in['wv'], 'A_wo': _A_in['wo'], 'B_x': _B_in['x'], 'B_w1': _B_in['w1'], 'B_w2': _B_in['w2'], 'c': _w((lambda *s: _rng.normal(s) * 0.05)(1, 640)), 'w_mod': _w((lambda *s: _rng.normal(s) * 0.05)(640, 6 * 640) * 640 ** (-0.5))}

def _fwd_reference(A_x, A_wq, A_wk, A_wv, A_wo, B_x, B_w1, B_w2, c, w_mod):

    def _A_ref(x, wq, wk, wv, wo):
        B, S, D = x.shape
        H = 32
        Dh = D // H
        q = (lambda x, *d: x.transpose(*d))((x @ wq).reshape(B, S, H, Dh), 0, 2, 1, 3)
        k = x @ wk
        v = x @ wv
        scores = jnp.einsum('bhqd,bkd->bhqk', q, k) * Dh ** (-0.5)
        p = _softmax(scores, axis=-1)
        o = jnp.einsum('bhqk,bkd->bhqd', p, v)
        return (lambda x, *d: x.transpose(*d))(o, 0, 2, 1, 3).reshape(B, S, H * Dh) @ wo

    def _B_ref(x, w1, w2):
        h = jnp.einsum('bsd,df->bsf', x, w1)
        h = _silu(h)
        out = jnp.einsum('bsf,fd->bsd', h, w2)
        return out
    x = A_x
    mod = (_silu(c) @ w_mod).reshape(c.shape[0], 6, 1, -1)
    sa, ca, ga, sb, cb, gb = (mod[:, 0].copy(), mod[:, 1].copy(), mod[:, 2].copy(), mod[:, 3].copy(), mod[:, 4].copy(), mod[:, 5].copy())
    h = _layernorm(x, axis=-1) * (1 + ca) + sa
    x = x + ga * _A_ref(h, A_wq, A_wk, A_wv, A_wo)
    h = _layernorm(x, axis=-1) * (1 + cb) + sb
    x = x + gb * _B_ref(h, B_w1, B_w2)
    return x

def setup_inputs():
    _inp = _fwd_setup_inputs()
    _gk = jax.random.fold_in(jax.random.key(int.from_bytes(__import__("os").urandom(4), "little")), 2 ** 31 - 1)
    _shapes = [[1, 2048, 640]]
    _dtypes = ['bfloat16']
    _gks = jax.random.split(_gk, len(_shapes))
    _gs = [jax.random.normal(k, s, dtype=jnp.dtype(d)) * 0.05 for k, s, d in zip(_gks, _shapes, _dtypes)]
    _inp['grad_out'] = _gs[0]
    return _inp

def reference(A_x, A_wq, A_wk, A_wv, A_wo, B_w1, B_w2, c, w_mod, B_x, grad_out):
    _const = dict(B_x=B_x)

    def _f(*_d):
        return _fwd_reference(**{'A_x': _d[0], 'A_wq': _d[1], 'A_wk': _d[2], 'A_wv': _d[3], 'A_wo': _d[4], 'B_w1': _d[5], 'B_w2': _d[6], 'c': _d[7], 'w_mod': _d[8], **_const})
    _out, _vjp = jax.vjp(_f, A_x, A_wq, A_wk, A_wv, A_wo, B_w1, B_w2, c, w_mod)
    _grads = _vjp(grad_out)
    _out0 = jnp.asarray(_out)
    return (_out0, *[jnp.asarray(_g) for _g in _grads])
```

```python
import math

import jax
import jax.numpy as jnp
import jax.experimental.pallas as pl
import jax.experimental.pallas.tpu as pltpu

S = 2048
D = 640
H = 32
DH = 20
F = 1728
TQ = 256
NB = S // TQ
NQ = TQ // 128
CH = 256
NC = S // CH
KT = CH // 128
HPF = 2
HPB = 2
LEAD = 1
EPS = 1e-5
SCALE = DH ** -0.5
LOG2E = math.log2(math.e)
LN2 = math.log(2.0)

f32 = jnp.float32
bf16 = jnp.bfloat16
u32 = jnp.uint32
NT = (((1,), (1,)), ((), ()))


def _dot(a, b):
    return jnp.dot(a, b, preferred_element_type=f32)


def _dot_nt(a, b):
    return jax.lax.dot_general(a, b, NT, preferred_element_type=f32)


def _sigmoid(x):
    return 1.0 / (1.0 + jnp.exp(-x))


def _wide(m):
    return jnp.concatenate([m] * NQ, axis=1)


def _fold(a):
    r = a[:, 0:128]
    for j in range(1, NQ):
        r = r + a[:, j * 128:(j + 1) * 128]
    return r


def _kernel(x_hbm, wq_hbm, wkT_ref, wvT_ref, wo_hbm, w1T_hbm, w2_hbm, c_ref, wmod_hbm, g_hbm,
            out_hbm, dx_hbm, dwq_hbm, dwkT_ref, dwvT_ref, dwo_hbm, dw1T_hbm, dw2_hbm, dc_ref, dwmod_hbm,
            x_ref, g_ref, wq_ref, wo_ref, w1T, w2_ref, wmod_ref,
            modc, wqT, woT, w1_ref, w2T, wkv, wkvT, xT, st, h1T, qTp, kT, vT1, kN, vN1,
            s_scr, p_scr, m_scr, mp_scr, oT, linv, doT, w_scr, dqT,
            dkT, dvT, dxT, dwq_a, dwo_a, dw1_a, dw2_a, dmod_a, dsc_s,
            sem_x, sem_in, sem_out, sem_dx, sem_w):
    MA = 2 * D

    def rows_of(b):
        return pl.ds(pl.multiple_of(b * TQ, TQ), TQ)

    def cp_x(b):
        return pltpu.make_async_copy(x_hbm.at[rows_of(b)], x_ref.at[rows_of(b)], sem_x.at[b])

    def cp_out(b):
        return pltpu.make_async_copy(x_ref.at[rows_of(b)], out_hbm.at[rows_of(b)], sem_out.at[b])

    def cp_dx(b):
        return pltpu.make_async_copy(g_ref.at[rows_of(b)], dx_hbm.at[rows_of(b)], sem_dx.at[b])

    cp_wma = pltpu.make_async_copy(wmod_hbm.at[:, 0:MA], wmod_ref.at[:, 0:MA], sem_in.at[0])
    cp_wq = pltpu.make_async_copy(wq_hbm, wq_ref, sem_in.at[1])
    cp_wmb = pltpu.make_async_copy(wmod_hbm.at[:, MA:6 * D], wmod_ref.at[:, MA:6 * D], sem_in.at[2])
    cp_wo = pltpu.make_async_copy(wo_hbm, wo_ref, sem_in.at[3])
    cp_w1 = pltpu.make_async_copy(w1T_hbm, w1T, sem_in.at[4])
    cp_w2 = pltpu.make_async_copy(w2_hbm, w2_ref, sem_in.at[5])
    cp_g = pltpu.make_async_copy(g_hbm, g_ref, sem_in.at[6])
    co_wq = pltpu.make_async_copy(wq_ref, dwq_hbm, sem_w.at[0])
    co_wo = pltpu.make_async_copy(wo_ref, dwo_hbm, sem_w.at[1])
    co_w1 = pltpu.make_async_copy(w1T, dw1T_hbm, sem_w.at[2])
    co_w2 = pltpu.make_async_copy(w2_ref, dw2_hbm, sem_w.at[3])
    co_wma = pltpu.make_async_copy(wmod_ref.at[:, 0:MA], dwmod_hbm.at[:, 0:MA], sem_w.at[4])
    co_wmb = pltpu.make_async_copy(wmod_ref.at[:, MA:6 * D], dwmod_hbm.at[:, MA:6 * D], sem_w.at[5])

    cp_wma.start()
    for b in range(NB):
        cp_x(b).start()
    cp_wq.start()

    c = c_ref[...].astype(f32)
    sig_c = _sigmoid(c)
    sc = c * sig_c
    sc16 = jnp.broadcast_to(sc, (16, D)).astype(bf16)

    wkvT[...] = jnp.zeros((128, D), bf16)
    wkvT[0:DH, :] = wkT_ref[...]
    wkvT[32:32 + DH, :] = wvT_ref[...]
    wkv[...] = wkvT[...].T

    dkT[...] = jnp.zeros_like(dkT)
    dvT[...] = jnp.zeros_like(dvT)
    dwq_a[...] = jnp.zeros_like(dwq_a)
    dwo_a[...] = jnp.zeros_like(dwo_a)
    dw1_a[...] = jnp.zeros_like(dw1_a)
    dw2_a[...] = jnp.zeros_like(dw2_a)
    dmod_a[...] = jnp.zeros_like(dmod_a)
    st[...] = jnp.zeros_like(st)

    def set_modc(js):
        mod = _dot(sc16, wmod_ref[:, js[0] * D:(js[-1] + 1) * D])
        for j in js:
            jj = j - js[0]
            mj = jnp.broadcast_to(mod[0:1, jj * D:(jj + 1) * D], (128, D))
            if j in (1, 4):
                mj = mj + 1.0
            modc[j] = mj.T

    cp_wma.wait()
    set_modc([0, 1])
    cp_wq.wait()
    cp_wmb.start()
    cp_wo.start()
    cp_w1.start()
    cp_w2.start()
    cp_g.start()
    wqT[...] = wq_ref[...].T

    row32 = jax.lax.broadcasted_iota(jnp.int32, (32, TQ), 0)

    def pro_blk(b, carry):
        cols = pl.ds(pl.multiple_of(b * TQ, TQ), TQ)
        cp_x(b).wait()
        xt = x_ref[cols, :].T
        xT[:, cols] = xt
        xf = xt.astype(f32)
        mu = jnp.mean(xf, axis=0, keepdims=True)
        xc = xf - mu
        var = jnp.mean(xc * xc, axis=0, keepdims=True)
        rstd = jax.lax.rsqrt(var + EPS)
        st[0:1, cols] = mu
        st[1:2, cols] = rstd
        h1 = (xc * rstd) * _wide(modc[1]) + _wide(modc[0])
        h1b = h1.astype(bf16)
        h1T[:, cols] = h1b
        q = _dot(wqT[...], h1b) * (SCALE * LOG2E)
        qz = jnp.concatenate([q, jnp.zeros((16, TQ), f32)], axis=0)
        for h in range(H):
            qh = jnp.where(row32 < DH, qz[DH * h:DH * h + 32, :], 0.0)
            qTp[h, :, cols] = qh.astype(bf16)
        kv = _dot(wkvT[0:64, :], h1b)
        k_t = kv[0:32, :]
        v_t = kv[32:64, :]
        kT[:, cols] = k_t.astype(bf16)
        vT1[:, cols] = jnp.where(row32 == DH, 1.0, v_t).astype(bf16)
        z96 = jnp.zeros((96, TQ), f32)
        kN[cols, :] = jnp.concatenate([k_t, z96], axis=0).T.astype(bf16)
        v11 = jnp.where((row32 == DH) | (row32 == DH + 1), 1.0, v_t)
        vN1[cols, :] = jnp.concatenate([v11, z96], axis=0).T.astype(bf16)
        return carry

    jax.lax.fori_loop(0, NB, pro_blk, 0)

    cp_wmb.wait()
    set_modc([2, 3, 4, 5])
    cp_wo.wait()
    woT[...] = wo_ref[...].T
    cp_w1.wait()
    w1_ref[...] = w1T[...].T
    cp_w2.wait()
    w2T[...] = w2_ref[...].T
    cp_g.wait()

    def stage_a(qt, slot, cc, mx):
        for kk in range(KT):
            r0 = cc * CH + kk * 128
            kblk = kN[r0:r0 + 128, 0:32]
            for qq in range(NQ):
                s = _dot(kblk, qt[:, qq * 128:(qq + 1) * 128])
                s_scr[slot, r0:r0 + 128, qq * 128:(qq + 1) * 128] = s
                sm = jnp.max(s.reshape(16, 8, 128), axis=0)
                mx[qq] = sm if mx[qq] is None else jnp.maximum(mx[qq], sm)

    def finish_max(slot, mx):
        for qq in range(NQ):
            m = jnp.max(mx[qq], axis=0, keepdims=True)
            m_scr[slot, :, qq * 128:(qq + 1) * 128] = jnp.broadcast_to(m, (8, 128))

    mx0 = [None] * NQ
    q00 = qTp[0, :, 0:TQ]
    for cc in range(NC):
        stage_a(q00, 0, cc, mx0)
    finish_max(0, mx0)
    mx1 = [None] * NQ
    q01 = qTp[1, :, 0:TQ]
    for cc in range(LEAD):
        stage_a(q01, 1, cc, mx1)
    for qq in range(NQ):
        mp_scr[:, qq * 128:(qq + 1) * 128] = mx1[qq]

    def finish_mod(j0, j1):
        rows = []
        for j in range(j0, j1):
            t = dmod_a[j].T
            rows.append(jnp.sum(t, axis=0, keepdims=True))
        dmod = jnp.concatenate(rows, axis=1)
        n = (j1 - j0) * D
        hi = dmod.astype(bf16).astype(f32)
        lo = dmod - hi
        r16 = jax.lax.broadcasted_iota(jnp.int32, (16, n), 0)
        dm16 = jnp.where(r16 == 0, hi, jnp.where(r16 == 1, lo, 0.0)).astype(bf16)
        dsc = _dot_nt(dm16, wmod_ref[:, j0 * D:j1 * D])
        scc = jnp.broadcast_to(sc, (128, D)).T
        for j in range(n // 128):
            wmod_ref[:, j0 * D + j * 128:j0 * D + (j + 1) * 128] = (
                scc * dmod[:, j * 128:(j + 1) * 128]).astype(bf16)
        return dsc

    def block(b, carry):
        cols = pl.ds(pl.multiple_of(b * TQ, TQ), TQ)
        bnext = jnp.minimum(b + 1, NB - 1)

        def fwd_iter(i, carry):
            h0 = i * HPF
            T = HPF * NC
            qslab = {}
            for j in range(1, HPF + 2):
                hh = h0 + j
                wrap = hh >= H
                hq = jnp.where(wrap, hh - H, hh)
                bq = jnp.where(wrap, bnext, b)
                qslab[j] = qTp[hq, :, pl.ds(pl.multiple_of(bq * TQ, TQ), TQ)]
            mx = {1: [mp_scr[:, qq * 128:(qq + 1) * 128] for qq in range(NQ)]}
            for j in range(2, HPF + 2):
                mx[j] = [None] * NQ
            pvals = {}
            acc = {}
            outs = {}

            def stage_b(t):
                j, cc = divmod(t, NC)
                slot = j % 2
                vals = {}
                for kk in range(KT):
                    r0 = cc * CH + kk * 128
                    for qq in range(NQ):
                        m = m_scr[slot, 0:1, qq * 128:(qq + 1) * 128]
                        p = jnp.exp2(s_scr[slot, r0:r0 + 128, qq * 128:(qq + 1) * 128] - m).astype(bf16)
                        p_scr[h0 + j, qq, r0 // 2:r0 // 2 + 64, :] = pltpu.bitcast(p, u32)
                        vals[(kk, qq)] = p
                pvals[t] = vals

            def stage_c(t):
                j, cc = divmod(t, NC)
                vals = pvals.pop(t)
                for kk in range(KT):
                    r0 = cc * CH + kk * 128
                    vblk = vT1[:, r0:r0 + 128]
                    for qq in range(NQ):
                        r = _dot(vblk, vals[(kk, qq)])
                        acc[(j, qq)] = r if (j, qq) not in acc else acc[(j, qq)] + r
                if cc == NC - 1:
                    a = jnp.concatenate([acc.pop((j, qq)) for qq in range(NQ)], axis=1)
                    li = 1.0 / a[DH:DH + 1, :]
                    linv[pl.ds(h0 + j, 1), :] = li
                    outs[j] = a[0:DH, :] * li
                    if j % 2 == 1:
                        pair = jnp.concatenate([outs[j - 1], outs[j]], axis=0)
                        r = pl.multiple_of((h0 + j - 1) * DH, 8)
                        oT[pl.ds(r, 2 * DH), :] = pair

            for t in range(T + 1):
                if t < T:
                    ta = t + NC + LEAD
                    ja, ca = divmod(ta, NC)
                    stage_a(qslab[ja], ja % 2, ca, mx[ja])
                    if ca == NC - 1:
                        finish_max(ja % 2, mx[ja])
                    stage_b(t)
                if t >= 1:
                    stage_c(t - 1)
            for qq in range(NQ):
                mp_scr[:, qq * 128:(qq + 1) * 128] = mx[HPF + 1][qq]
            return carry

        jax.lax.fori_loop(0, H // HPF, fwd_iter, 0)

        sa_w, ca_w, ga_w = _wide(modc[0]), _wide(modc[1]), _wide(modc[2])
        sb_w, cb_w, gb_w = _wide(modc[3]), _wide(modc[4]), _wide(modc[5])
        o = oT[...]
        ob = o.astype(bf16)
        a = _dot(woT[...], ob)
        x1 = xT[:, cols].astype(f32) + ga_w * a
        mu2 = jnp.mean(x1, axis=0, keepdims=True)
        xc2 = x1 - mu2
        var2 = jnp.mean(xc2 * xc2, axis=0, keepdims=True)
        rstd2 = jax.lax.rsqrt(var2 + EPS)
        xh2 = xc2 * rstd2
        h2b = (xh2 * cb_w + sb_w).astype(bf16)
        u = _dot(w1T[...], h2b)
        sg = _sigmoid(u)
        sb16 = (u * sg).astype(bf16)
        f = _dot(w2T[...], sb16)
        outT = x1 + gb_w * f
        x_ref[cols, :] = outT.astype(bf16).T
        cp_out(b).start()
        gT = g_ref[cols, :].T.astype(f32)
        dmod_a[5] += _fold(gT * f)
        dfb = (gT * gb_w).astype(bf16)
        dw2_a[...] += _dot_nt(sb16, dfb)
        dsT = _dot(w2_ref[...], dfb)
        dub = (dsT * (sg * (1.0 + u * (1.0 - sg)))).astype(bf16)
        dw1_a[...] += _dot_nt(dub, h2b)
        dh2 = _dot(w1_ref[...], dub)
        dmod_a[3] += _fold(dh2)
        dmod_a[4] += _fold(dh2 * xh2)
        dxh2 = dh2 * cb_w
        dx1 = gT + rstd2 * (dxh2 - jnp.mean(dxh2, axis=0, keepdims=True)
                            - xh2 * jnp.mean(dxh2 * xh2, axis=0, keepdims=True))
        dmod_a[2] += _fold(dx1 * a)
        dab = (dx1 * ga_w).astype(bf16)
        dwo_a[...] += _dot_nt(ob, dab)
        doT[...] = _dot(wo_ref[...], dab)
        dxT[:, cols] = dx1

        @pl.when(b == NB - 1)
        def _():
            wo_ref[...] = dwo_a[...].astype(bf16)
            co_wo.start()
            w1T[...] = dw1_a[...].astype(bf16)
            co_w1.start()
            w2_ref[...] = dw2_a[...].astype(bf16)
            co_w2.start()
            dsc_s[...] = finish_mod(2, 6)
            co_wmb.start()

        def w_pair(i, carry):
            r = pl.multiple_of(i * 2 * DH, 8)
            dpair = doT[pl.ds(r, 2 * DH), :]
            opair = oT[pl.ds(r, 2 * DH), :]
            for j in range(2):
                dd = dpair[j * DH:(j + 1) * DH, :]
                oo = opair[j * DH:(j + 1) * DH, :]
                li = linv[pl.ds(2 * i + j, 1), :]
                nd = -jnp.sum(dd * oo, axis=0, keepdims=True) * li
                hi = nd.astype(bf16).astype(f32)
                lo = nd - hi
                w = jnp.concatenate([dd * li, hi, lo, jnp.zeros((10, TQ), f32)], axis=0)
                w_scr[2 * i + j] = w.astype(bf16)
            return carry

        jax.lax.fori_loop(0, H // 2, w_pair, 0)

        def bwd_iter(i, carry):
            h0 = i * HPB
            T = HPB * NC
            ws = {j: w_scr[h0 + j] for j in range(HPB)}
            qs = {j: qTp[h0 + j, :, cols] for j in range(HPB)}
            dsv = {}
            dqs = {}
            outs = {}

            def stage1(t):
                j, cc = divmod(t, NC)
                vals = {}
                for kk in range(KT):
                    r0 = cc * CH + kk * 128
                    vblk = vN1[r0:r0 + 128, 0:32]
                    for qq in range(NQ):
                        dp = _dot(vblk, ws[j][:, qq * 128:(qq + 1) * 128])
                        p = pltpu.bitcast(p_scr[h0 + j, qq, r0 // 2:r0 // 2 + 64, :], bf16)
                        vals[(kk, qq)] = (p.astype(f32) * dp).astype(bf16)
                dsv[t] = vals

            def stage2(t):
                j, cc = divmod(t, NC)
                ds = dsv.pop(t)
                for kk in range(KT):
                    r0 = cc * CH + kk * 128
                    a2 = None
                    for qq in range(NQ):
                        p = pltpu.bitcast(p_scr[h0 + j, qq, r0 // 2:r0 // 2 + 64, :], bf16)
                        r = _dot_nt(ws[j][:, qq * 128:(qq + 1) * 128], p)
                        a2 = r if a2 is None else a2 + r
                    dvT[:, r0:r0 + 128] += a2
                for kk in range(KT):
                    r0 = cc * CH + kk * 128
                    a2 = None
                    for qq in range(NQ):
                        r = _dot_nt(qs[j][:, qq * 128:(qq + 1) * 128], ds[(kk, qq)])
                        a2 = r if a2 is None else a2 + r
                    dkT[:, r0:r0 + 128] += a2
                for kk in range(KT):
                    r0 = cc * CH + kk * 128
                    kblk = kT[:, r0:r0 + 128]
                    for qq in range(NQ):
                        r = _dot(kblk, ds[(kk, qq)])
                        dqs[(j, qq)] = r if (j, qq) not in dqs else dqs[(j, qq)] + r
                if cc == NC - 1:
                    a3 = jnp.concatenate([dqs.pop((j, qq)) for qq in range(NQ)], axis=1)
                    outs[j] = a3[0:DH, :]
                    if j % 2 == 1:
                        pair = jnp.concatenate([outs[j - 1], outs[j]], axis=0)
                        r = pl.multiple_of((h0 + j - 1) * DH, 8)
                        dqT[pl.ds(r, 2 * DH), :] = pair

            for t in range(T + 1):
                if t < T:
                    stage1(t)
                if t >= 1:
                    stage2(t - 1)
            return carry

        jax.lax.fori_loop(0, H // HPB, bwd_iter, 0)

        dqb = (dqT[...] * SCALE).astype(bf16)
        h1b = h1T[:, cols]
        dwq_a[...] += _dot_nt(h1b, dqb)
        dh1 = _dot(wq_ref[...], dqb)
        mu = st[0:1, cols]
        rstd = st[1:2, cols]
        xh1 = (xT[:, cols].astype(f32) - mu) * rstd
        dmod_a[0] += _fold(dh1)
        dmod_a[1] += _fold(dh1 * xh1)
        dxh = dh1 * ca_w
        dxT[:, cols] += rstd * (dxh - jnp.mean(dxh, axis=0, keepdims=True)
                                - xh1 * jnp.mean(dxh * xh1, axis=0, keepdims=True))
        return carry

    jax.lax.fori_loop(0, NB, block, 0)

    wq_ref[...] = dwq_a[...].astype(bf16)
    co_wq.start()
    row32s = jax.lax.broadcasted_iota(jnp.int32, (32, S), 0)
    dk = jnp.where(row32s < DH, dkT[...] * LN2, 0.0).astype(bf16)
    dv = jnp.where(row32s < DH, dvT[...], 0.0).astype(bf16)
    dkv = jnp.concatenate([dk, dv], axis=0)
    dwkv = _dot_nt(dkv, h1T[...])
    dwkT_ref[...] = dwkv[0:DH, :].astype(bf16)
    dwvT_ref[...] = dwkv[32:32 + DH, :].astype(bf16)
    kT[...] = dk
    vT1[...] = dv

    def epi_blk(b, carry):
        cols = pl.ds(pl.multiple_of(b * TQ, TQ), TQ)
        dkvb = jnp.concatenate([kT[:, cols], vT1[:, cols]], axis=0)
        dh1 = _dot(wkv[:, 0:64], dkvb)
        mu = st[0:1, cols]
        rstd = st[1:2, cols]
        xh1 = (xT[:, cols].astype(f32) - mu) * rstd
        dmod_a[0] += _fold(dh1)
        dmod_a[1] += _fold(dh1 * xh1)
        dxh = dh1 * _wide(modc[1])
        dxf = dxT[:, cols] + rstd * (dxh - jnp.mean(dxh, axis=0, keepdims=True)
                                     - xh1 * jnp.mean(dxh * xh1, axis=0, keepdims=True))
        g_ref[cols, :] = dxf.astype(bf16).T
        cp_dx(b).start()
        return carry

    jax.lax.fori_loop(0, NB, epi_blk, 0)

    dsc = finish_mod(0, 2) + dsc_s[...]
    co_wma.start()
    dsc = dsc[0:1, :] + dsc[1:2, :]
    dc_ref[...] = (dsc * (sig_c * (1.0 + c * (1.0 - sig_c)))).astype(bf16)

    for b in range(NB):
        cp_out(b).wait()
    co_wo.wait()
    co_w1.wait()
    co_w2.wait()
    co_wmb.wait()
    co_wq.wait()
    for b in range(NB):
        cp_dx(b).wait()
    co_wma.wait()


@jax.jit
def pallas_adaLN_cond__grouped_kv_mqa__dense_activation_silu__prompt_kernel(
    A_x: jax.Array,
    A_wq: jax.Array,
    A_wk: jax.Array,
    A_wv: jax.Array,
    A_wo: jax.Array,
    B_x: jax.Array,
    B_w1: jax.Array,
    B_w2: jax.Array,
    c: jax.Array,
    w_mod: jax.Array,
    grad_out: jax.Array,
):
    x = A_x.reshape(S, D)
    g = grad_out.reshape(S, D)
    sds = jax.ShapeDtypeStruct
    out_shape = (
        sds((S, D), bf16), sds((S, D), bf16), sds((D, D), bf16), sds((DH, D), bf16), sds((DH, D), bf16),
        sds((D, D), bf16), sds((F, D), bf16), sds((F, D), bf16), sds((1, D), bf16), sds((D, 6 * D), bf16),
    )
    hbm = pl.BlockSpec(memory_space=pl.ANY)
    vm = pl.BlockSpec(memory_space=pltpu.VMEM)
    in_specs = [hbm, hbm, vm, vm, hbm, hbm, hbm, vm, hbm, hbm]
    out_specs = (hbm, hbm, hbm, vm, vm, hbm, hbm, hbm, vm, hbm)
    V = pltpu.VMEM
    scratch = [
        V((S, D), bf16),
        V((S, D), bf16),
        V((D, D), bf16),
        V((D, D), bf16),
        V((F, D), bf16),
        V((F, D), bf16),
        V((D, 6 * D), bf16),
        V((6, D, 128), f32),
        V((D, D), bf16),
        V((D, D), bf16),
        V((D, F), bf16),
        V((D, F), bf16),
        V((D, 128), bf16),
        V((128, D), bf16),
        V((D, S), bf16),
        V((8, S), f32),
        V((D, S), bf16),
        V((H, 32, S), bf16),
        V((32, S), bf16),
        V((32, S), bf16),
        V((S, 128), bf16),
        V((S, 128), bf16),
        V((2, S, TQ), f32),
        V((H, NQ, S // 2, 128), u32),
        V((2, 8, TQ), f32),
        V((8, TQ), f32),
        V((D, TQ), f32),
        V((H, TQ), f32),
        V((D, TQ), f32),
        V((H, 32, TQ), bf16),
        V((D, TQ), f32),
        V((32, S), f32),
        V((32, S), f32),
        V((D, S), f32),
        V((D, D), f32),
        V((D, D), f32),
        V((F, D), f32),
        V((F, D), f32),
        V((6, D, 128), f32),
        V((16, D), f32),
        pltpu.SemaphoreType.DMA((NB,)),
        pltpu.SemaphoreType.DMA((7,)),
        pltpu.SemaphoreType.DMA((NB,)),
        pltpu.SemaphoreType.DMA((NB,)),
        pltpu.SemaphoreType.DMA((6,)),
    ]
    res = pl.pallas_call(
        _kernel,
        out_shape=out_shape,
        in_specs=in_specs,
        out_specs=out_specs,
        scratch_shapes=scratch,
        compiler_params=pltpu.CompilerParams(vmem_limit_bytes=126 * 1024 * 1024),
    )(x, A_wq, A_wk.T, A_wv.T, A_wo, B_w1.T, B_w2, c, w_mod, g)
    out, dx = res[0].reshape(1, S, D), res[1].reshape(1, S, D)
    return (out, dx, res[2], res[3].T, res[4].T, res[5], res[6].T, res[7], res[8], res[9])
```

```python
import math

import jax
import jax.numpy as jnp
import jax.experimental.pallas as pl
import jax.experimental.pallas.tpu as pltpu

S = 2048
D = 640
H = 32
DH = 20
F = 1728
TQ = 256
NB = S // TQ
NQ = TQ // 128
CH = 256
NC = S // CH
KT = CH // 128
HPF = 8
HPB = 8
LEAD = 1
EPS = 1e-5
SCALE = DH ** -0.5
LOG2E = math.log2(math.e)
LN2 = math.log(2.0)

f32 = jnp.float32
bf16 = jnp.bfloat16
u32 = jnp.uint32
NT = (((1,), (1,)), ((), ()))


def _dot(a, b):
    return jnp.dot(a, b, preferred_element_type=f32)


def _dot_nt(a, b):
    return jax.lax.dot_general(a, b, NT, preferred_element_type=f32)


def _sigmoid(x):
    return 1.0 / (1.0 + jnp.exp(-x))


def _wide(m):
    return jnp.concatenate([m] * NQ, axis=1)


def _fold(a):
    r = a[:, 0:128]
    for j in range(1, NQ):
        r = r + a[:, j * 128:(j + 1) * 128]
    return r


def _rows_loop(n_rows, chunk, fn):
    assert n_rows % chunk == 0

    def body(i, carry):
        fn(pl.ds(pl.multiple_of(i * chunk, chunk), chunk))
        return carry

    jax.lax.fori_loop(0, n_rows // chunk, body, 0)


def _zero(ref, chunk):
    def fn(r):
        ref[r, :] = jnp.zeros((chunk, ref.shape[1]), ref.dtype)
    _rows_loop(ref.shape[0], chunk, fn)


def _cast_to(dst, src, chunk):
    def fn(r):
        dst[r, :] = src[r, :].astype(dst.dtype)
    _rows_loop(src.shape[0], chunk, fn)


def _transpose_to(dst, src):
    def body(i, carry):
        cs = pl.ds(pl.multiple_of(i * 128, 128), 128)
        dst[cs, :] = src[:, cs].T
        return carry
    jax.lax.fori_loop(0, src.shape[1] // 128, body, 0)


def _kernel(x_hbm, wq_hbm, wkT_ref, wvT_ref, wo_hbm, w1T_hbm, w2_hbm, c_ref, wmod_hbm, g_hbm,
            out_hbm, dx_hbm, dwq_hbm, dwkT_ref, dwvT_ref, dwo_hbm, dw1T_hbm, dw2_hbm, dc_ref, dwmod_hbm,
            x_ref, g_ref, wq_ref, wo_ref, w1T, w2_ref, wmod_ref,
            modc, wqT, woT, w1_ref, w2T, wkv, wkvT, xT, st, h1T, qTp, kT, vT1, kN, vN1,
            s_scr, p_scr, m_scr, mp_scr, oT, linv, doT, w_scr, dqT,
            dkT, dvT, dxT, dwq_a, dwo_a, dw1_a, dw2_a, dmod_a, dsc_s, row_s, scc_s,
            sem_x, sem_in, sem_out, sem_dx, sem_w):
    MA = 2 * D

    def rows_of(b):
        return pl.ds(pl.multiple_of(b * TQ, TQ), TQ)

    def cp_x(b):
        return pltpu.make_async_copy(x_hbm.at[rows_of(b)], x_ref.at[rows_of(b)], sem_x.at[b])

    def cp_out(b):
        return pltpu.make_async_copy(x_ref.at[rows_of(b)], out_hbm.at[rows_of(b)], sem_out.at[b])

    def cp_dx(b):
        return pltpu.make_async_copy(g_ref.at[rows_of(b)], dx_hbm.at[rows_of(b)], sem_dx.at[b])

    cp_wma = pltpu.make_async_copy(wmod_hbm.at[:, 0:MA], wmod_ref.at[:, 0:MA], sem_in.at[0])
    cp_wq = pltpu.make_async_copy(wq_hbm, wq_ref, sem_in.at[1])
    cp_wmb = pltpu.make_async_copy(wmod_hbm.at[:, MA:6 * D], wmod_ref.at[:, MA:6 * D], sem_in.at[2])
    cp_wo = pltpu.make_async_copy(wo_hbm, wo_ref, sem_in.at[3])
    cp_w1 = pltpu.make_async_copy(w1T_hbm, w1T, sem_in.at[4])
    cp_w2 = pltpu.make_async_copy(w2_hbm, w2_ref, sem_in.at[5])
    cp_g = pltpu.make_async_copy(g_hbm, g_ref, sem_in.at[6])
    co_wq = pltpu.make_async_copy(wq_ref, dwq_hbm, sem_w.at[0])
    co_wo = pltpu.make_async_copy(wo_ref, dwo_hbm, sem_w.at[1])
    co_w1 = pltpu.make_async_copy(w1T, dw1T_hbm, sem_w.at[2])
    co_w2 = pltpu.make_async_copy(w2_ref, dw2_hbm, sem_w.at[3])
    co_wma = pltpu.make_async_copy(wmod_ref.at[:, 0:MA], dwmod_hbm.at[:, 0:MA], sem_w.at[4])
    co_wmb = pltpu.make_async_copy(wmod_ref.at[:, MA:6 * D], dwmod_hbm.at[:, MA:6 * D], sem_w.at[5])

    cp_wma.start()
    cp_x(0).start()
    cp_wq.start()

    c = c_ref[...].astype(f32)
    sig_c = _sigmoid(c)
    sc = c * sig_c
    sc16 = jnp.broadcast_to(sc, (16, D)).astype(bf16)

    wkvT[...] = jnp.zeros((128, D), bf16)
    wkvT[0:DH, :] = wkT_ref[...]
    wkvT[32:32 + DH, :] = wvT_ref[...]
    wkv[...] = wkvT[...].T

    dkT[...] = jnp.zeros_like(dkT)
    dvT[...] = jnp.zeros_like(dvT)
    _zero(dwq_a, 64)
    _zero(dwo_a, 64)
    _zero(dw1_a, 64)
    _zero(dw2_a, 64)
    for j in range(6):
        dmod_a[j] = jnp.zeros((D, 128), f32)
    st[...] = jnp.zeros_like(st)
    _zero(dxT, 16)
    dqT[...] = jnp.zeros_like(dqT)

    def set_modc(js):
        mod = _dot(sc16, wmod_ref[:, js[0] * D:(js[-1] + 1) * D])
        for j in js:
            jj = j - js[0]
            mj = jnp.broadcast_to(mod[0:1, jj * D:(jj + 1) * D], (128, D))
            if j in (1, 4):
                mj = mj + 1.0
            modc[j] = mj.T

    cp_wma.wait()
    for b in range(1, NB):
        cp_x(b).start()
    set_modc([0, 1])
    cp_wq.wait()
    _transpose_to(wqT, wq_ref)

    row32 = jax.lax.broadcasted_iota(jnp.int32, (32, TQ), 0)

    def ln_blk(b):
        cols = pl.ds(pl.multiple_of(b * TQ, TQ), TQ)
        xT[:, cols] = x_ref[cols, :].T
        RC = 64
        acc = None
        for r in range(0, D, RC):
            blk = xT[r:r + RC, cols].astype(f32)
            part = jnp.sum(blk.reshape(RC // 8, 8, TQ), axis=0)
            acc = part if acc is None else acc + part
        mu = jnp.sum(acc, axis=0, keepdims=True) * (1.0 / D)
        acc = None
        for r in range(0, D, RC):
            blk = xT[r:r + RC, cols].astype(f32) - mu
            part = jnp.sum((blk * blk).reshape(RC // 8, 8, TQ), axis=0)
            acc = part if acc is None else acc + part
        var = jnp.sum(acc, axis=0, keepdims=True) * (1.0 / D)
        rstd = jax.lax.rsqrt(var + EPS)
        st[0:1, cols] = mu
        st[1:2, cols] = rstd
        for r in range(0, D, RC):
            blk = (xT[r:r + RC, cols].astype(f32) - mu) * rstd
            h1 = blk * _wide(modc[1, r:r + RC, :]) + _wide(modc[0, r:r + RC, :])
            h1T[r:r + RC, cols] = h1.astype(bf16)

    def proj_blk(b):
        cols = pl.ds(pl.multiple_of(b * TQ, TQ), TQ)
        h1b = h1T[:, cols]
        kv = _dot(wkvT[0:64, :], h1b)
        k_t = kv[0:32, :]
        v_t = kv[32:64, :]
        kT[:, cols] = k_t.astype(bf16)
        vT1[:, cols] = jnp.where(row32 == DH, 1.0, v_t).astype(bf16)
        z96 = jnp.zeros((96, TQ), f32)
        kN[cols, :] = jnp.concatenate([k_t, z96], axis=0).T.astype(bf16)
        v11 = jnp.where((row32 == DH) | (row32 == DH + 1), 1.0, v_t)
        vN1[cols, :] = jnp.concatenate([v11, z96], axis=0).T.astype(bf16)
        QC = 8
        for qc in range(H // QC):
            q = _dot(wqT[qc * QC * DH:(qc + 1) * QC * DH, :], h1b) * (SCALE * LOG2E)
            qz = jnp.concatenate([q, jnp.zeros((16, TQ), f32)], axis=0)
            for h in range(QC):
                qh = jnp.where(row32 < DH, qz[DH * h:DH * h + 32, :], 0.0)
                qTp[qc * QC + h, :, cols] = qh.astype(bf16)

    cp_x(0).wait()
    ln_blk(0)

    def pro_blk(b, carry):
        @pl.when(b + 1 < NB)
        def _():
            cp_x(b + 1).wait()

        @pl.when(b == 1)
        def _():
            cp_wo.start()
            cp_w1.start()
            cp_w2.start()
        proj_blk(b)
        ln_blk(jnp.minimum(b + 1, NB - 1))
        return carry

    jax.lax.fori_loop(0, NB, pro_blk, 0)

    cp_wmb.start()
    cp_g.start()
    cp_wo.wait()
    cp_w1.wait()
    cp_w2.wait()

    def tr_body(i, carry):
        cs = pl.ds(pl.multiple_of(i * 128, 128), 128)
        woT[cs, :] = wo_ref[:, cs].T
        w1_ref[cs, :] = w1T[:, cs].T
        w2T[cs, :] = w2_ref[:, cs].T
        return carry

    jax.lax.fori_loop(0, D // 128, tr_body, 0)

    def stage_a(qt, slot, cc, mx):
        for kk in range(KT):
            r0 = cc * CH + kk * 128
            kblk = kN[r0:r0 + 128, 0:32]
            for qq in range(NQ):
                s = _dot(kblk, qt[:, qq * 128:(qq + 1) * 128])
                s_scr[slot, r0:r0 + 128, qq * 128:(qq + 1) * 128] = s
                sm = jnp.max(s.reshape(16, 8, 128), axis=0)
                mx[qq] = sm if mx[qq] is None else jnp.maximum(mx[qq], sm)

    def finish_max(slot, mx):
        for qq in range(NQ):
            m = jnp.max(mx[qq], axis=0, keepdims=True)
            m_scr[slot, :, qq * 128:(qq + 1) * 128] = jnp.broadcast_to(m, (8, 128))

    mx0 = [None] * NQ
    q00 = qTp[0, :, 0:TQ]
    for cc in range(NC):
        stage_a(q00, 0, cc, mx0)
    finish_max(0, mx0)
    mx1 = [None] * NQ
    q01 = qTp[1, :, 0:TQ]
    for cc in range(LEAD):
        stage_a(q01, 1, cc, mx1)
    for qq in range(NQ):
        mp_scr[:, qq * 128:(qq + 1) * 128] = mx1[qq]

    def finish_mod(j0, j1):
        rows = []
        for j in range(j0, j1):
            t = dmod_a[j].T
            rows.append(jnp.sum(t, axis=0, keepdims=True))
        dmod = jnp.concatenate(rows, axis=1)
        n = (j1 - j0) * D
        hi = dmod.astype(bf16).astype(f32)
        lo = dmod - hi
        r16 = jax.lax.broadcasted_iota(jnp.int32, (16, n), 0)
        dm16 = jnp.where(r16 == 0, hi, jnp.where(r16 == 1, lo, 0.0)).astype(bf16)
        dsc = _dot_nt(dm16, wmod_ref[:, j0 * D:j1 * D])
        row_s[0:1, j0 * D:j1 * D] = dmod
        scc_s[...] = jnp.broadcast_to(sc, (128, D)).T

        def body(i, carry):
            cs = pl.ds(pl.multiple_of(j0 * D + i * 128, 128), 128)
            wmod_ref[:, cs] = (scc_s[...] * row_s[0:1, cs]).astype(bf16)
            return carry

        jax.lax.fori_loop(0, n // 128, body, 0)
        return dsc

    def qproj_bwd(b, hh):
        lc = pl.ds(pl.multiple_of(hh * 128, 128), 128)
        cols = pl.ds(pl.multiple_of(b * TQ + hh * 128, 128), 128)
        dqb = (dqT[:, lc] * SCALE).astype(bf16)
        h1b = h1T[:, cols]
        dwq_a[...] += _dot_nt(h1b, dqb)
        dh1 = _dot(wq_ref[...], dqb)
        mu = st[0:1, cols]
        rstd = st[1:2, cols]
        xh1 = (xT[:, cols].astype(f32) - mu) * rstd
        dmod_a[0] += dh1
        dmod_a[1] += dh1 * xh1
        dxh = dh1 * modc[1]
        dxT[:, cols] += rstd * (dxh - jnp.mean(dxh, axis=0, keepdims=True)
                                - xh1 * jnp.mean(dxh * xh1, axis=0, keepdims=True))

    def block(b, carry):
        cols = pl.ds(pl.multiple_of(b * TQ, TQ), TQ)
        bnext = jnp.minimum(b + 1, NB - 1)

        def fwd_iter(i, carry):
            h0 = i * HPF
            T = HPF * NC
            qslab = {}
            for j in range(1, HPF + 2):
                hh = h0 + j
                wrap = hh >= H
                hq = jnp.where(wrap, hh - H, hh)
                bq = jnp.where(wrap, bnext, b)
                qslab[j] = qTp[hq, :, pl.ds(pl.multiple_of(bq * TQ, TQ), TQ)]
            mx = {1: [mp_scr[:, qq * 128:(qq + 1) * 128] for qq in range(NQ)]}
            for j in range(2, HPF + 2):
                mx[j] = [None] * NQ
            pvals = {}
            acc = {}
            outs = {}

            def stage_b(t):
                j, cc = divmod(t, NC)
                slot = j % 2
                vals = {}
                for kk in range(KT):
                    r0 = cc * CH + kk * 128
                    for qq in range(NQ):
                        m = m_scr[slot, 0:1, qq * 128:(qq + 1) * 128]
                        e = jnp.exp2(s_scr[slot, r0:r0 + 128, qq * 128:(qq + 1) * 128] - m)
                        p = e.astype(bf16)
                        p_scr[h0 + j, qq, r0:r0 + 64, :] = e[0:64].astype(bf16)
                        p_scr[h0 + j, qq, r0 + 64:r0 + 128, :] = e[64:128].astype(bf16)
                        vals[(kk, qq)] = p
                pvals[t] = vals

            def stage_c(t):
                j, cc = divmod(t, NC)
                vals = pvals.pop(t)
                for kk in range(KT):
                    r0 = cc * CH + kk * 128
                    vblk = vT1[:, r0:r0 + 128]
                    for qq in range(NQ):
                        r = _dot(vblk, vals[(kk, qq)])
                        acc[(j, qq)] = r if (j, qq) not in acc else acc[(j, qq)] + r
                if cc == NC - 1:
                    a = jnp.concatenate([acc.pop((j, qq)) for qq in range(NQ)], axis=1)
                    li = 1.0 / a[DH:DH + 1, :]
                    linv[pl.ds(h0 + j, 1), :] = li
                    outs[j] = a[0:DH, :] * li
                    if j % 2 == 1:
                        pair = jnp.concatenate([outs[j - 1], outs[j]], axis=0)
                        r = pl.multiple_of((h0 + j - 1) * DH, 8)
                        oT[pl.ds(r, 2 * DH), :] = pair

            for t in range(T + 1):
                if t < T:
                    ta = t + NC + LEAD
                    ja, ca = divmod(ta, NC)
                    stage_a(qslab[ja], ja % 2, ca, mx[ja])
                    if ca == NC - 1:
                        finish_max(ja % 2, mx[ja])
                    stage_b(t)
                if t >= 1:
                    stage_c(t - 1)
            for qq in range(NQ):
                mp_scr[:, qq * 128:(qq + 1) * 128] = mx[HPF + 1][qq]
            return carry

        jax.lax.fori_loop(0, H // HPF, fwd_iter, 0)

        bprev = jnp.maximum(b - 1, 0)

        @pl.when(b == 0)
        def _():
            cp_wmb.wait()
            set_modc([2, 3, 4, 5])
            cp_g.wait()

        def dense_half(hh, carry):
            lc = pl.ds(pl.multiple_of(hh * 128, 128), 128)
            gc = pl.ds(pl.multiple_of(b * TQ + hh * 128, 128), 128)
            ga_w, sb_w, cb_w, gb_w = modc[2], modc[3], modc[4], modc[5]
            o = oT[:, lc]
            ob = o.astype(bf16)
            gT = g_ref[gc, :].T.astype(f32)
            dfb = (gT * gb_w).astype(bf16)
            a = _dot(woT[...], ob)
            dsT = _dot(w2_ref[...], dfb)
            x1 = xT[:, gc].astype(f32) + ga_w * a
            mu2 = jnp.mean(x1, axis=0, keepdims=True)
            xc2 = x1 - mu2
            var2 = jnp.mean(xc2 * xc2, axis=0, keepdims=True)
            rstd2 = jax.lax.rsqrt(var2 + EPS)
            xh2 = xc2 * rstd2
            h2b = (xh2 * cb_w + sb_w).astype(bf16)
            u = _dot(w1T[...], h2b)
            qproj_bwd(bprev, hh)
            sg = _sigmoid(u)
            sb16 = (u * sg).astype(bf16)
            dub = (dsT * (sg * (1.0 + u * (1.0 - sg)))).astype(bf16)
            dh2 = _dot(w1_ref[...], dub)
            f = _dot(w2T[...], sb16)
            dmod_a[3] += dh2
            dmod_a[4] += dh2 * xh2
            dxh2 = dh2 * cb_w
            dx1 = gT + rstd2 * (dxh2 - jnp.mean(dxh2, axis=0, keepdims=True)
                                - xh2 * jnp.mean(dxh2 * xh2, axis=0, keepdims=True))
            dmod_a[2] += dx1 * a
            dab = (dx1 * ga_w).astype(bf16)
            do = _dot(wo_ref[...], dab)
            dw2_a[...] += _dot_nt(sb16, dfb)
            dw1_a[...] += _dot_nt(dub, h2b)
            dwo_a[...] += _dot_nt(ob, dab)
            outT = x1 + gb_w * f
            x_ref[gc, :] = outT.astype(bf16).T
            dmod_a[5] += gT * f
            dxT[:, gc] += dx1
            for h in range(H):
                li = linv[h:h + 1, lc]
                wr = (do[h * DH:(h + 1) * DH, :] * li).astype(bf16).astype(f32)
                nd = -jnp.sum(wr * o[h * DH:(h + 1) * DH, :], axis=0, keepdims=True)
                hi = nd.astype(bf16).astype(f32)
                lo = nd - hi
                w = jnp.concatenate([wr, hi, lo, jnp.zeros((10, 128), f32)], axis=0)
                w_scr[h, :, lc] = w.astype(bf16)
            return carry

        jax.lax.fori_loop(0, NQ, dense_half, 0)
        cp_out(b).start()

        @pl.when(b == NB - 1)
        def _():
            _cast_to(wo_ref, dwo_a, 64)
            co_wo.start()
            _cast_to(w1T, dw1_a, 64)
            co_w1.start()
            _cast_to(w2_ref, dw2_a, 64)
            co_w2.start()

        def bwd_iter(i, carry):
            h0 = i * HPB
            T = HPB * NC
            ws = {j: w_scr[h0 + j] for j in range(HPB)}
            qs = {j: qTp[h0 + j, :, cols] for j in range(HPB)}
            dsv = {}
            dqs = {}
            outs = {}

            def stage1(t):
                j, cc = divmod(t, NC)
                vals = {}
                for kk in range(KT):
                    r0 = cc * CH + kk * 128
                    vblk = vN1[r0:r0 + 128, 0:32]
                    for qq in range(NQ):
                        dp = _dot(vblk, ws[j][:, qq * 128:(qq + 1) * 128])
                        p = p_scr[h0 + j, qq, r0:r0 + 128, :]
                        vals[(kk, qq)] = (p.astype(f32) * dp).astype(bf16)
                dsv[t] = vals

            def stage2(t):
                j, cc = divmod(t, NC)
                ds = dsv.pop(t)
                for kk in range(KT):
                    r0 = cc * CH + kk * 128
                    a2 = None
                    for qq in range(NQ):
                        p = p_scr[h0 + j, qq, r0:r0 + 128, :]
                        r = _dot_nt(ws[j][:, qq * 128:(qq + 1) * 128], p)
                        a2 = r if a2 is None else a2 + r
                    dvT[:, r0:r0 + 128] += a2
                for kk in range(KT):
                    r0 = cc * CH + kk * 128
                    a2 = None
                    for qq in range(NQ):
                        r = _dot_nt(qs[j][:, qq * 128:(qq + 1) * 128], ds[(kk, qq)])
                        a2 = r if a2 is None else a2 + r
                    dkT[:, r0:r0 + 128] += a2
                for kk in range(KT):
                    r0 = cc * CH + kk * 128
                    kblk = kT[:, r0:r0 + 128]
                    for qq in range(NQ):
                        r = _dot(kblk, ds[(kk, qq)])
                        dqs[(j, qq)] = r if (j, qq) not in dqs else dqs[(j, qq)] + r
                if cc == NC - 1:
                    a3 = jnp.concatenate([dqs.pop((j, qq)) for qq in range(NQ)], axis=1)
                    outs[j] = a3[0:DH, :]
                    if j % 2 == 1:
                        pair = jnp.concatenate([outs[j - 1], outs[j]], axis=0)
                        r = pl.multiple_of((h0 + j - 1) * DH, 8)
                        dqT[pl.ds(r, 2 * DH), :] = pair

            for t in range(T + 1):
                if t < T:
                    stage1(t)
                if t >= 1:
                    stage2(t - 1)
            return carry

        jax.lax.fori_loop(0, H // HPB, bwd_iter, 0)

        return carry

    jax.lax.fori_loop(0, NB, block, 0)

    dsc_s[...] = finish_mod(2, 6)
    co_wmb.start()
    for hh in range(NQ):
        qproj_bwd(NB - 1, hh)
    _cast_to(wq_ref, dwq_a, 64)
    co_wq.start()
    row32s = jax.lax.broadcasted_iota(jnp.int32, (32, S), 0)
    dk = jnp.where(row32s < DH, dkT[...] * LN2, 0.0).astype(bf16)
    dv = jnp.where(row32s < DH, dvT[...], 0.0).astype(bf16)
    dkv = jnp.concatenate([dk, dv], axis=0)
    dwkv = _dot_nt(dkv, h1T[...])
    dwkT_ref[...] = dwkv[0:DH, :].astype(bf16)
    dwvT_ref[...] = dwkv[32:32 + DH, :].astype(bf16)
    kT[...] = dk
    vT1[...] = dv

    def epi_blk(b, carry):
        cols = pl.ds(pl.multiple_of(b * TQ, TQ), TQ)
        dkvb = jnp.concatenate([kT[:, cols], vT1[:, cols]], axis=0)
        dh1 = _dot(wkv[:, 0:64], dkvb)
        mu = st[0:1, cols]
        rstd = st[1:2, cols]
        xh1 = (xT[:, cols].astype(f32) - mu) * rstd
        dmod_a[0] += _fold(dh1)
        dmod_a[1] += _fold(dh1 * xh1)
        dxh = dh1 * _wide(modc[1])
        dxf = dxT[:, cols] + rstd * (dxh - jnp.mean(dxh, axis=0, keepdims=True)
                                     - xh1 * jnp.mean(dxh * xh1, axis=0, keepdims=True))
        g_ref[cols, :] = dxf.astype(bf16).T
        cp_dx(b).start()
        return carry

    jax.lax.fori_loop(0, NB, epi_blk, 0)

    dsc = finish_mod(0, 2) + dsc_s[...]
    co_wma.start()
    dsc = dsc[0:1, :] + dsc[1:2, :]
    dc_ref[...] = (dsc * (sig_c * (1.0 + c * (1.0 - sig_c)))).astype(bf16)

    for b in range(NB):
        cp_out(b).wait()
    co_wo.wait()
    co_w1.wait()
    co_w2.wait()
    co_wmb.wait()
    co_wq.wait()
    for b in range(NB):
        cp_dx(b).wait()
    co_wma.wait()


@jax.jit
def pallas_adaLN_cond__grouped_kv_mqa__dense_activation_silu__prompt_kernel(
    A_x: jax.Array,
    A_wq: jax.Array,
    A_wk: jax.Array,
    A_wv: jax.Array,
    A_wo: jax.Array,
    B_x: jax.Array,
    B_w1: jax.Array,
    B_w2: jax.Array,
    c: jax.Array,
    w_mod: jax.Array,
    grad_out: jax.Array,
):
    x = A_x.reshape(S, D)
    g = grad_out.reshape(S, D)
    sds = jax.ShapeDtypeStruct
    out_shape = (
        sds((S, D), bf16), sds((S, D), bf16), sds((D, D), bf16), sds((DH, D), bf16), sds((DH, D), bf16),
        sds((D, D), bf16), sds((F, D), bf16), sds((F, D), bf16), sds((1, D), bf16), sds((D, 6 * D), bf16),
    )
    hbm = pl.BlockSpec(memory_space=pl.ANY)
    vm = pl.BlockSpec(memory_space=pltpu.VMEM)
    in_specs = [hbm, hbm, vm, vm, hbm, hbm, hbm, vm, hbm, hbm]
    out_specs = (hbm, hbm, hbm, vm, vm, hbm, hbm, hbm, vm, hbm)
    V = pltpu.VMEM
    scratch = [
        V((S, D), bf16),
        V((S, D), bf16),
        V((D, D), bf16),
        V((D, D), bf16),
        V((F, D), bf16),
        V((F, D), bf16),
        V((D, 6 * D), bf16),
        V((6, D, 128), f32),
        V((D, D), bf16),
        V((D, D), bf16),
        V((D, F), bf16),
        V((D, F), bf16),
        V((D, 128), bf16),
        V((128, D), bf16),
        V((D, S), bf16),
        V((8, S), f32),
        V((D, S), bf16),
        V((H, 32, S), bf16),
        V((32, S), bf16),
        V((32, S), bf16),
        V((S, 128), bf16),
        V((S, 128), bf16),
        V((2, S, TQ), f32),
        V((H, NQ, S, 128), bf16),
        V((2, 8, TQ), f32),
        V((8, TQ), f32),
        V((D, TQ), f32),
        V((H, TQ), f32),
        V((D, TQ), f32),
        V((H, 32, TQ), bf16),
        V((D, TQ), f32),
        V((32, S), f32),
        V((32, S), f32),
        V((D, S), f32),
        V((D, D), f32),
        V((D, D), f32),
        V((F, D), f32),
        V((F, D), f32),
        V((6, D, 128), f32),
        V((16, D), f32),
        V((8, 6 * D), f32),
        V((D, 128), f32),
        pltpu.SemaphoreType.DMA((NB,)),
        pltpu.SemaphoreType.DMA((7,)),
        pltpu.SemaphoreType.DMA((NB,)),
        pltpu.SemaphoreType.DMA((NB,)),
        pltpu.SemaphoreType.DMA((6,)),
    ]
    res = pl.pallas_call(
        _kernel,
        out_shape=out_shape,
        in_specs=in_specs,
        out_specs=out_specs,
        scratch_shapes=scratch,
        compiler_params=pltpu.CompilerParams(vmem_limit_bytes=126 * 1024 * 1024),
    )(x, A_wq, A_wk.T, A_wv.T, A_wo, B_w1.T, B_w2, c, w_mod, g)
    out, dx = res[0].reshape(1, S, D), res[1].reshape(1, S, D)
    return (out, dx, res[2], res[3].T, res[4].T, res[5], res[6].T, res[7], res[8], res[9])
```

```python
import math

import jax
import jax.numpy as jnp
import jax.experimental.pallas as pl
import jax.experimental.pallas.tpu as pltpu

S = 2048
D = 640
H = 32
DH = 20
F = 1728
TQ = 256
NB = S // TQ
NQ = TQ // 128
CH = 256
NC = S // CH
KT = CH // 128
HPF = 8
HPB = 8
LEAD = 1
EPS = 1e-5
SCALE = DH ** -0.5
LOG2E = math.log2(math.e)
LN2 = math.log(2.0)

f32 = jnp.float32
bf16 = jnp.bfloat16
u32 = jnp.uint32
NT = (((1,), (1,)), ((), ()))


def _dot(a, b):
    return jnp.dot(a, b, preferred_element_type=f32)


def _dot_nt(a, b):
    return jax.lax.dot_general(a, b, NT, preferred_element_type=f32)


def _sigmoid(x):
    return 1.0 / (1.0 + jnp.exp(-x))


def _wide(m):
    return jnp.concatenate([m] * NQ, axis=1)


def _fold(a):
    r = a[:, 0:128]
    for j in range(1, NQ):
        r = r + a[:, j * 128:(j + 1) * 128]
    return r


def _rows_loop(n_rows, chunk, fn):
    assert n_rows % chunk == 0

    def body(i, carry):
        fn(pl.ds(pl.multiple_of(i * chunk, chunk), chunk))
        return carry

    jax.lax.fori_loop(0, n_rows // chunk, body, 0)


def _zero(ref, chunk):
    def fn(r):
        ref[r, :] = jnp.zeros((chunk, ref.shape[1]), ref.dtype)
    _rows_loop(ref.shape[0], chunk, fn)


def _cast_to(dst, src, chunk):
    def fn(r):
        dst[r, :] = src[r, :].astype(dst.dtype)
    _rows_loop(src.shape[0], chunk, fn)


def _transpose_to(dst, src):
    def body(i, carry):
        cs = pl.ds(pl.multiple_of(i * 128, 128), 128)
        dst[cs, :] = src[:, cs].T
        return carry
    jax.lax.fori_loop(0, src.shape[1] // 128, body, 0)


def _kernel(x_hbm, wq_hbm, wkT_ref, wvT_ref, wo_hbm, w1T_hbm, w2_hbm, c_ref, wmod_hbm, g_hbm,
            out_hbm, dx_hbm, dwq_hbm, dwkT_ref, dwvT_ref, dwo_hbm, dw1T_hbm, dw2_hbm, dc_ref, dwmod_hbm,
            x_ref, g_ref, wq_ref, wo_ref, w1T, w2_ref, wmod_ref,
            modc, wqT, woT, w1_ref, w2T, wkv, wkvT, xT, st, h1T, qTp, kT, vT1, kN, vN1,
            s_scr, p_scr, m_scr, mp_scr, oT, linv, dh1q, w_scr, dqT,
            dkT, dvT, dxT, dwq_a, dwo_a, dw1_a, dw2_a, dmod_a, dsc_s, row_s, scc_s, dqb_s, dwkv_a,
            sem_x, sem_in, sem_out, sem_dx, sem_w):
    MA = 2 * D

    def rows_of(b):
        return pl.ds(pl.multiple_of(b * TQ, TQ), TQ)

    def cp_x(b):
        return pltpu.make_async_copy(x_hbm.at[rows_of(b)], x_ref.at[rows_of(b)], sem_x.at[b])

    def cp_out(b):
        return pltpu.make_async_copy(x_ref.at[rows_of(b)], out_hbm.at[rows_of(b)], sem_out.at[b])

    def cp_dx(b):
        return pltpu.make_async_copy(g_ref.at[rows_of(b)], dx_hbm.at[rows_of(b)], sem_dx.at[b])

    cp_wma = pltpu.make_async_copy(wmod_hbm.at[:, 0:MA], wmod_ref.at[:, 0:MA], sem_in.at[0])
    cp_wq = pltpu.make_async_copy(wq_hbm, wq_ref, sem_in.at[1])
    cp_wmb = pltpu.make_async_copy(wmod_hbm.at[:, MA:6 * D], wmod_ref.at[:, MA:6 * D], sem_in.at[2])
    cp_wo = pltpu.make_async_copy(wo_hbm, wo_ref, sem_in.at[3])
    cp_w1 = pltpu.make_async_copy(w1T_hbm, w1T, sem_in.at[4])
    cp_w2 = pltpu.make_async_copy(w2_hbm, w2_ref, sem_in.at[5])
    cp_g = pltpu.make_async_copy(g_hbm, g_ref, sem_in.at[6])
    co_wq = pltpu.make_async_copy(wq_ref, dwq_hbm, sem_w.at[0])
    co_wo = pltpu.make_async_copy(wo_ref, dwo_hbm, sem_w.at[1])
    co_w1 = pltpu.make_async_copy(w1T, dw1T_hbm, sem_w.at[2])
    co_w2 = pltpu.make_async_copy(w2_ref, dw2_hbm, sem_w.at[3])
    co_wma = pltpu.make_async_copy(wmod_ref.at[:, 0:MA], dwmod_hbm.at[:, 0:MA], sem_w.at[4])
    co_wmb = pltpu.make_async_copy(wmod_ref.at[:, MA:6 * D], dwmod_hbm.at[:, MA:6 * D], sem_w.at[5])

    cp_wma.start()
    cp_x(0).start()
    cp_wq.start()

    c = c_ref[...].astype(f32)
    sig_c = _sigmoid(c)
    sc = c * sig_c
    sc16 = jnp.broadcast_to(sc, (16, D)).astype(bf16)

    wkvT[...] = jnp.zeros((128, D), bf16)
    wkvT[0:DH, :] = wkT_ref[...]
    wkvT[32:32 + DH, :] = wvT_ref[...]
    wkv[...] = wkvT[...].T

    dkT[...] = jnp.zeros_like(dkT)
    dvT[...] = jnp.zeros_like(dvT)
    _zero(dwq_a, 64)
    _zero(dwo_a, 64)
    _zero(dw1_a, 64)
    _zero(dw2_a, 64)
    for j in range(6):
        dmod_a[j] = jnp.zeros((D, 128), f32)
    st[...] = jnp.zeros_like(st)
    dqT[...] = jnp.zeros_like(dqT)

    def set_modc(js):
        mod = _dot(sc16, wmod_ref[:, js[0] * D:(js[-1] + 1) * D])
        for j in js:
            jj = j - js[0]
            mj = jnp.broadcast_to(mod[0:1, jj * D:(jj + 1) * D], (128, D))
            if j in (1, 4):
                mj = mj + 1.0
            modc[j] = mj.T

    cp_wma.wait()
    for b in range(1, NB):
        cp_x(b).start()
    set_modc([0, 1])
    cp_wq.wait()
    _transpose_to(wqT, wq_ref)

    row32 = jax.lax.broadcasted_iota(jnp.int32, (32, TQ), 0)

    def ln_blk(b):
        cols = pl.ds(pl.multiple_of(b * TQ, TQ), TQ)
        xT[:, cols] = x_ref[cols, :].T
        RC = 64
        acc = None
        for r in range(0, D, RC):
            blk = xT[r:r + RC, cols].astype(f32)
            part = jnp.sum(blk.reshape(RC // 8, 8, TQ), axis=0)
            acc = part if acc is None else acc + part
        mu = jnp.sum(acc, axis=0, keepdims=True) * (1.0 / D)
        acc = None
        for r in range(0, D, RC):
            blk = xT[r:r + RC, cols].astype(f32) - mu
            part = jnp.sum((blk * blk).reshape(RC // 8, 8, TQ), axis=0)
            acc = part if acc is None else acc + part
        var = jnp.sum(acc, axis=0, keepdims=True) * (1.0 / D)
        rstd = jax.lax.rsqrt(var + EPS)
        st[0:1, cols] = mu
        st[1:2, cols] = rstd
        for r in range(0, D, RC):
            blk = (xT[r:r + RC, cols].astype(f32) - mu) * rstd
            h1 = blk * _wide(modc[1, r:r + RC, :]) + _wide(modc[0, r:r + RC, :])
            h1T[r:r + RC, cols] = h1.astype(bf16)

    def proj_blk(b):
        cols = pl.ds(pl.multiple_of(b * TQ, TQ), TQ)
        h1b = h1T[:, cols]
        kv = _dot(wkvT[0:64, :], h1b)
        k_t = kv[0:32, :]
        v_t = kv[32:64, :]
        kT[:, cols] = k_t.astype(bf16)
        vT1[:, cols] = jnp.where(row32 == DH, 1.0, v_t).astype(bf16)
        z96 = jnp.zeros((96, TQ), f32)
        hc = pl.ds(pl.multiple_of(b * (TQ // 2), TQ // 2), TQ // 2)
        kN[hc, :] = pltpu.bitcast(jnp.concatenate([k_t, z96], axis=0).T.astype(bf16), u32)
        v11 = jnp.where((row32 == DH) | (row32 == DH + 1), 1.0, v_t)
        vN1[hc, :] = pltpu.bitcast(jnp.concatenate([v11, z96], axis=0).T.astype(bf16), u32)
        QC = 8
        for qc in range(H // QC):
            q = _dot(wqT[qc * QC * DH:(qc + 1) * QC * DH, :], h1b) * (SCALE * LOG2E)
            qz = jnp.concatenate([q, jnp.zeros((16, TQ), f32)], axis=0)
            for h in range(QC):
                qh = jnp.where(row32 < DH, qz[DH * h:DH * h + 32, :], 0.0)
                qTp[qc * QC + h, :, cols] = qh.astype(bf16)

    cp_x(0).wait()
    ln_blk(0)

    def pro_blk(b, carry):
        @pl.when(b + 1 < NB)
        def _():
            cp_x(b + 1).wait()

        @pl.when(b == 1)
        def _():
            cp_wo.start()
            cp_w1.start()
            cp_w2.start()
        proj_blk(b)
        ln_blk(jnp.minimum(b + 1, NB - 1))
        return carry

    jax.lax.fori_loop(0, NB, pro_blk, 0)

    cp_wmb.start()
    cp_g.start()
    cp_wo.wait()
    cp_w1.wait()
    cp_w2.wait()

    def tr_body(i, carry):
        cs = pl.ds(pl.multiple_of(i * 128, 128), 128)
        woT[cs, :] = wo_ref[:, cs].T
        w1_ref[cs, :] = w1T[:, cs].T
        w2T[cs, :] = w2_ref[:, cs].T
        return carry

    jax.lax.fori_loop(0, D // 128, tr_body, 0)

    def stage_a(qt, slot, cc, mx):
        for kk in range(KT):
            r0 = cc * CH + kk * 128
            kblk = pltpu.bitcast(kN[r0 // 2:r0 // 2 + 64, :], bf16)[:, 0:32]
            for qq in range(NQ):
                s = _dot(kblk, qt[:, qq * 128:(qq + 1) * 128])
                s_scr[slot, r0:r0 + 128, qq * 128:(qq + 1) * 128] = s
                sm = jnp.max(s.reshape(16, 8, 128), axis=0)
                mx[qq] = sm if mx[qq] is None else jnp.maximum(mx[qq], sm)

    def finish_max(slot, mx):
        for qq in range(NQ):
            m = jnp.max(mx[qq], axis=0, keepdims=True)
            m_scr[slot, :, qq * 128:(qq + 1) * 128] = jnp.broadcast_to(m, (8, 128))

    mx0 = [None] * NQ
    q00 = qTp[0, :, 0:TQ]
    for cc in range(NC):
        stage_a(q00, 0, cc, mx0)
    finish_max(0, mx0)
    mx1 = [None] * NQ
    q01 = qTp[1, :, 0:TQ]
    for cc in range(LEAD):
        stage_a(q01, 1, cc, mx1)
    for qq in range(NQ):
        mp_scr[:, qq * 128:(qq + 1) * 128] = mx1[qq]

    def finish_mod(j0, j1):
        rows = []
        for j in range(j0, j1):
            t = dmod_a[j].T
            rows.append(jnp.sum(t, axis=0, keepdims=True))
        dmod = jnp.concatenate(rows, axis=1)
        n = (j1 - j0) * D
        hi = dmod.astype(bf16).astype(f32)
        lo = dmod - hi
        r16 = jax.lax.broadcasted_iota(jnp.int32, (16, n), 0)
        dm16 = jnp.where(r16 == 0, hi, jnp.where(r16 == 1, lo, 0.0)).astype(bf16)
        dsc = _dot_nt(dm16, wmod_ref[:, j0 * D:j1 * D])
        row_s[0:1, j0 * D:j1 * D] = dmod
        scc_s[...] = jnp.broadcast_to(sc, (128, D)).T

        def body(i, carry):
            cs = pl.ds(pl.multiple_of(j0 * D + i * 128, 128), 128)
            wmod_ref[:, cs] = (scc_s[...] * row_s[0:1, cs]).astype(bf16)
            return carry

        jax.lax.fori_loop(0, n // 128, body, 0)
        return dsc

    def qproj_bwd(b, hh):
        lc = pl.ds(pl.multiple_of(hh * 128, 128), 128)
        cols = pl.ds(pl.multiple_of(b * TQ + hh * 128, 128), 128)
        dqb = (dqT[:, lc] * SCALE).astype(bf16)
        dwq_a[...] += _dot_nt(h1T[:, cols], dqb)
        dh1q[:, cols] = _dot(wq_ref[...], dqb)

    def block(b, carry):
        cols = pl.ds(pl.multiple_of(b * TQ, TQ), TQ)
        bnext = jnp.minimum(b + 1, NB - 1)

        def fwd_iter(i, carry):
            h0 = i * HPF
            T = HPF * NC
            qslab = {}
            for j in range(1, HPF + 2):
                hh = h0 + j
                wrap = hh >= H
                hq = jnp.where(wrap, hh - H, hh)
                bq = jnp.where(wrap, bnext, b)
                qslab[j] = qTp[hq, :, pl.ds(pl.multiple_of(bq * TQ, TQ), TQ)]
            mx = {1: [mp_scr[:, qq * 128:(qq + 1) * 128] for qq in range(NQ)]}
            for j in range(2, HPF + 2):
                mx[j] = [None] * NQ
            pvals = {}
            acc = {}
            outs = {}

            def stage_b(t):
                j, cc = divmod(t, NC)
                slot = j % 2
                vals = {}
                for kk in range(KT):
                    r0 = cc * CH + kk * 128
                    for qq in range(NQ):
                        m = m_scr[slot, 0:1, qq * 128:(qq + 1) * 128]
                        e = jnp.exp2(s_scr[slot, r0:r0 + 128, qq * 128:(qq + 1) * 128] - m)
                        p = e.astype(bf16)
                        p_scr[h0 + j, qq, r0:r0 + 64, :] = e[0:64].astype(bf16)
                        p_scr[h0 + j, qq, r0 + 64:r0 + 128, :] = e[64:128].astype(bf16)
                        vals[(kk, qq)] = p
                pvals[t] = vals

            def stage_c(t):
                j, cc = divmod(t, NC)
                vals = pvals.pop(t)
                for kk in range(KT):
                    r0 = cc * CH + kk * 128
                    vblk = vT1[:, r0:r0 + 128]
                    for qq in range(NQ):
                        r = _dot(vblk, vals[(kk, qq)])
                        acc[(j, qq)] = r if (j, qq) not in acc else acc[(j, qq)] + r
                if cc == NC - 1:
                    a = jnp.concatenate([acc.pop((j, qq)) for qq in range(NQ)], axis=1)
                    li = 1.0 / a[DH:DH + 1, :]
                    linv[pl.ds(h0 + j, 1), :] = li
                    outs[j] = a[0:DH, :] * li
                    if j % 2 == 1:
                        pair = jnp.concatenate([outs[j - 1], outs[j]], axis=0)
                        r = pl.multiple_of((h0 + j - 1) * DH, 8)
                        oT[pl.ds(r, 2 * DH), :] = pair

            for t in range(T + 1):
                if t < T:
                    ta = t + NC + LEAD
                    ja, ca = divmod(ta, NC)
                    stage_a(qslab[ja], ja % 2, ca, mx[ja])
                    if ca == NC - 1:
                        finish_max(ja % 2, mx[ja])
                    stage_b(t)
                if t >= 1:
                    stage_c(t - 1)
            for qq in range(NQ):
                mp_scr[:, qq * 128:(qq + 1) * 128] = mx[HPF + 1][qq]
            return carry

        jax.lax.fori_loop(0, H // HPF, fwd_iter, 0)

        bprev = jnp.maximum(b - 1, 0)

        @pl.when(b == 0)
        def _():
            cp_wmb.wait()
            set_modc([2, 3, 4, 5])
            cp_g.wait()

        def dense_half(hh, carry):
            lc = pl.ds(pl.multiple_of(hh * 128, 128), 128)
            gc = pl.ds(pl.multiple_of(b * TQ + hh * 128, 128), 128)
            ga_w, sb_w, cb_w, gb_w = modc[2], modc[3], modc[4], modc[5]
            o = oT[:, lc]
            ob = o.astype(bf16)
            gT = g_ref[gc, :].T.astype(f32)
            dfb = (gT * gb_w).astype(bf16)
            a = _dot(woT[...], ob)
            dsT = _dot(w2_ref[...], dfb)
            x1 = xT[:, gc].astype(f32) + ga_w * a
            mu2 = jnp.mean(x1, axis=0, keepdims=True)
            xc2 = x1 - mu2
            var2 = jnp.mean(xc2 * xc2, axis=0, keepdims=True)
            rstd2 = jax.lax.rsqrt(var2 + EPS)
            xh2 = xc2 * rstd2
            h2b = (xh2 * cb_w + sb_w).astype(bf16)
            u = _dot(w1T[...], h2b)
            qproj_bwd(bprev, hh)
            sg = _sigmoid(u)
            sb16 = (u * sg).astype(bf16)
            dub = (dsT * (sg * (1.0 + u * (1.0 - sg)))).astype(bf16)
            dh2 = _dot(w1_ref[...], dub)
            f = _dot(w2T[...], sb16)
            dmod_a[3] += dh2
            dmod_a[4] += dh2 * xh2
            dxh2 = dh2 * cb_w
            dx1 = gT + rstd2 * (dxh2 - jnp.mean(dxh2, axis=0, keepdims=True)
                                - xh2 * jnp.mean(dxh2 * xh2, axis=0, keepdims=True))
            dmod_a[2] += dx1 * a
            dab = (dx1 * ga_w).astype(bf16)
            do = _dot(wo_ref[...], dab)
            dw2_a[...] += _dot_nt(sb16, dfb)
            dw1_a[...] += _dot_nt(dub, h2b)
            dwo_a[...] += _dot_nt(ob, dab)
            outT = x1 + gb_w * f
            x_ref[gc, :] = outT.astype(bf16).T
            dmod_a[5] += gT * f
            dxT[:, gc] = dx1
            for h in range(H):
                li = linv[h:h + 1, lc]
                wr = (do[h * DH:(h + 1) * DH, :] * li).astype(bf16).astype(f32)
                nd = -jnp.sum(wr * o[h * DH:(h + 1) * DH, :], axis=0, keepdims=True)
                hi = nd.astype(bf16).astype(f32)
                lo = nd - hi
                w = jnp.concatenate([wr, hi, lo, jnp.zeros((10, 128), f32)], axis=0)
                w_scr[h, :, lc] = w.astype(bf16)
            return carry

        jax.lax.fori_loop(0, NQ, dense_half, 0)
        cp_out(b).start()

        @pl.when(b == NB - 1)
        def _():
            _cast_to(wo_ref, dwo_a, 64)
            co_wo.start()
            _cast_to(w1T, dw1_a, 64)
            co_w1.start()
            _cast_to(w2_ref, dw2_a, 64)
            co_w2.start()

        def bwd_iter(i, carry):
            h0 = i * HPB
            T = HPB * NC
            ws = {j: w_scr[h0 + j] for j in range(HPB)}
            qs = {j: qTp[h0 + j, :, cols] for j in range(HPB)}
            dsv = {}
            dqs = {}
            outs = {}

            def stage1(t):
                j, cc = divmod(t, NC)
                vals = {}
                for kk in range(KT):
                    r0 = cc * CH + kk * 128
                    vblk = pltpu.bitcast(vN1[r0 // 2:r0 // 2 + 64, :], bf16)[:, 0:32]
                    for qq in range(NQ):
                        dp = _dot(vblk, ws[j][:, qq * 128:(qq + 1) * 128])
                        p = p_scr[h0 + j, qq, r0:r0 + 128, :]
                        vals[(kk, qq)] = (p.astype(f32) * dp).astype(bf16)
                dsv[t] = vals

            def stage2(t):
                j, cc = divmod(t, NC)
                ds = dsv.pop(t)
                for kk in range(KT):
                    r0 = cc * CH + kk * 128
                    a2 = None
                    for qq in range(NQ):
                        p = p_scr[h0 + j, qq, r0:r0 + 128, :]
                        r = _dot_nt(ws[j][:, qq * 128:(qq + 1) * 128], p)
                        a2 = r if a2 is None else a2 + r
                    dvT[:, r0:r0 + 128] += a2
                for kk in range(KT):
                    r0 = cc * CH + kk * 128
                    a2 = None
                    for qq in range(NQ):
                        r = _dot_nt(qs[j][:, qq * 128:(qq + 1) * 128], ds[(kk, qq)])
                        a2 = r if a2 is None else a2 + r
                    dkT[:, r0:r0 + 128] += a2
                for kk in range(KT):
                    r0 = cc * CH + kk * 128
                    kblk = kT[:, r0:r0 + 128]
                    for qq in range(NQ):
                        r = _dot(kblk, ds[(kk, qq)])
                        dqs[(j, qq)] = r if (j, qq) not in dqs else dqs[(j, qq)] + r
                if cc == NC - 1:
                    a3 = jnp.concatenate([dqs.pop((j, qq)) for qq in range(NQ)], axis=1)
                    outs[j] = a3[0:DH, :]
                    if j % 2 == 1:
                        pair = jnp.concatenate([outs[j - 1], outs[j]], axis=0)
                        r = pl.multiple_of((h0 + j - 1) * DH, 8)
                        dqT[pl.ds(r, 2 * DH), :] = pair

            for t in range(T + 1):
                if t < T:
                    stage1(t)
                if t >= 1:
                    stage2(t - 1)
            return carry

        jax.lax.fori_loop(0, H // HPB, bwd_iter, 0)

        return carry

    jax.lax.fori_loop(0, NB, block, 0)

    row32s = jax.lax.broadcasted_iota(jnp.int32, (32, S), 0)
    kT[...] = jnp.where(row32s < DH, dkT[...] * LN2, 0.0).astype(bf16)
    vT1[...] = jnp.where(row32s < DH, dvT[...], 0.0).astype(bf16)
    dqb_s[...] = (dqT[...] * SCALE).astype(bf16)
    dwkv_a[...] = jnp.zeros_like(dwkv_a)
    dsc_s[...] = finish_mod(2, 6)
    co_wmb.start()
    RQ = D // NB
    last = slice((NB - 1) * TQ, NB * TQ)

    def q_slice(k, live):
        rows = pl.ds(pl.multiple_of(k * RQ, 16), RQ)
        dqb = dqb_s[...]
        dh1q[rows, last] = _dot(wq_ref[rows, :], dqb)
        upd = _dot_nt(h1T[rows, last], dqb)
        dwq_a[rows, :] += upd if live is None else jnp.where(live, upd, 0.0)

    q_slice(0, None)

    def epi_blk(b, carry):
        cols = pl.ds(pl.multiple_of(b * TQ, TQ), TQ)
        dkvb = jnp.concatenate([kT[:, cols], vT1[:, cols]], axis=0)
        dh1 = _dot(wkv[:, 0:64], dkvb) + dh1q[:, cols]
        dwkv_a[...] += _dot_nt(dkvb, h1T[:, cols])
        q_slice(jnp.minimum(b + 1, NB - 1), b + 1 < NB)
        mu = st[0:1, cols]
        rstd = st[1:2, cols]
        xh1 = (xT[:, cols].astype(f32) - mu) * rstd
        dmod_a[0] += _fold(dh1)
        dmod_a[1] += _fold(dh1 * xh1)
        dxh = dh1 * _wide(modc[1])
        dxf = dxT[:, cols] + rstd * (dxh - jnp.mean(dxh, axis=0, keepdims=True)
                                     - xh1 * jnp.mean(dxh * xh1, axis=0, keepdims=True))
        g_ref[cols, :] = dxf.astype(bf16).T
        cp_dx(b).start()
        return carry

    jax.lax.fori_loop(0, NB, epi_blk, 0)
    _cast_to(wq_ref, dwq_a, 64)
    co_wq.start()
    dwkT_ref[...] = dwkv_a[0:DH, :].astype(bf16)
    dwvT_ref[...] = dwkv_a[32:32 + DH, :].astype(bf16)

    dsc = finish_mod(0, 2) + dsc_s[...]
    co_wma.start()
    dsc = dsc[0:1, :] + dsc[1:2, :]
    dc_ref[...] = (dsc * (sig_c * (1.0 + c * (1.0 - sig_c)))).astype(bf16)

    for b in range(NB):
        cp_out(b).wait()
    co_wo.wait()
    co_w1.wait()
    co_w2.wait()
    co_wmb.wait()
    co_wq.wait()
    for b in range(NB):
        cp_dx(b).wait()
    co_wma.wait()


@jax.jit
def pallas_adaLN_cond__grouped_kv_mqa__dense_activation_silu__prompt_kernel(
    A_x: jax.Array,
    A_wq: jax.Array,
    A_wk: jax.Array,
    A_wv: jax.Array,
    A_wo: jax.Array,
    B_x: jax.Array,
    B_w1: jax.Array,
    B_w2: jax.Array,
    c: jax.Array,
    w_mod: jax.Array,
    grad_out: jax.Array,
):
    x = A_x.reshape(S, D)
    g = grad_out.reshape(S, D)
    sds = jax.ShapeDtypeStruct
    out_shape = (
        sds((S, D), bf16), sds((S, D), bf16), sds((D, D), bf16), sds((DH, D), bf16), sds((DH, D), bf16),
        sds((D, D), bf16), sds((F, D), bf16), sds((F, D), bf16), sds((1, D), bf16), sds((D, 6 * D), bf16),
    )
    hbm = pl.BlockSpec(memory_space=pl.ANY)
    vm = pl.BlockSpec(memory_space=pltpu.VMEM)
    in_specs = [hbm, hbm, vm, vm, hbm, hbm, hbm, vm, hbm, hbm]
    out_specs = (hbm, hbm, hbm, vm, vm, hbm, hbm, hbm, vm, hbm)
    V = pltpu.VMEM
    scratch = [
        V((S, D), bf16),
        V((S, D), bf16),
        V((D, D), bf16),
        V((D, D), bf16),
        V((F, D), bf16),
        V((F, D), bf16),
        V((D, 6 * D), bf16),
        V((6, D, 128), f32),
        V((D, D), bf16),
        V((D, D), bf16),
        V((D, F), bf16),
        V((D, F), bf16),
        V((D, 128), bf16),
        V((128, D), bf16),
        V((D, S), bf16),
        V((8, S), f32),
        V((D, S), bf16),
        V((H, 32, S), bf16),
        V((32, S), bf16),
        V((32, S), bf16),
        V((S // 2, 128), u32),
        V((S // 2, 128), u32),
        V((2, S, TQ), f32),
        V((H, NQ, S, 128), bf16),
        V((2, 8, TQ), f32),
        V((8, TQ), f32),
        V((D, TQ), f32),
        V((H, TQ), f32),
        V((D, S), f32),
        V((H, 32, TQ), bf16),
        V((D, TQ), f32),
        V((32, S), f32),
        V((32, S), f32),
        V((D, S), f32),
        V((D, D), f32),
        V((D, D), f32),
        V((F, D), f32),
        V((F, D), f32),
        V((6, D, 128), f32),
        V((16, D), f32),
        V((8, 6 * D), f32),
        V((D, 128), f32),
        V((D, TQ), bf16),
        V((64, D), f32),
        pltpu.SemaphoreType.DMA((NB,)),
        pltpu.SemaphoreType.DMA((7,)),
        pltpu.SemaphoreType.DMA((NB,)),
        pltpu.SemaphoreType.DMA((NB,)),
        pltpu.SemaphoreType.DMA((6,)),
    ]
    res = pl.pallas_call(
        _kernel,
        out_shape=out_shape,
        in_specs=in_specs,
        out_specs=out_specs,
        scratch_shapes=scratch,
        compiler_params=pltpu.CompilerParams(vmem_limit_bytes=126 * 1024 * 1024),
    )(x, A_wq, A_wk.T, A_wv.T, A_wo, B_w1.T, B_w2, c, w_mod, g)
    out, dx = res[0].reshape(1, S, D), res[1].reshape(1, S, D)
    return (out, dx, res[2], res[3].T, res[4].T, res[5], res[6].T, res[7], res[8], res[9])
```

```python
import math

import jax
import jax.numpy as jnp
import jax.experimental.pallas as pl
import jax.experimental.pallas.tpu as pltpu

S = 2048
D = 640
H = 32
DH = 20
F = 1728
TQ = 256
NB = S // TQ
NQ = TQ // 128
CH = 256
NC = S // CH
KT = CH // 128
HPF = 8
HPB = 16
LEAD = 1
EPS = 1e-5
SCALE = DH ** -0.5
LOG2E = math.log2(math.e)
LN2 = math.log(2.0)

f32 = jnp.float32
bf16 = jnp.bfloat16
u32 = jnp.uint32
NT = (((1,), (1,)), ((), ()))
NN = (((1,), (0,)), ((), ()))
MR = 24


def _dot(a, b):
    return jax.lax.dot_general(a, b, NN, preferred_element_type=f32)


def _dot_nt(a, b):
    return jax.lax.dot_general(a, b, NT, preferred_element_type=f32)


def _pack2(a, b):
    ua = jax.lax.bitcast_convert_type(a, u32)
    ub = jax.lax.bitcast_convert_type(b, u32)
    return (ua >> 16) | (ub & jnp.uint32(0xFFFF0000))


def _pack_halves(a):
    return _pack2(a[0:64], a[64:128])


def _unpack_half(x, idx):
    y = (x << 16) if idx == 0 else (x & jnp.uint32(0xFFFF0000))
    return jax.lax.bitcast_convert_type(y, f32)


def _perm_matrix(inverse):
    r = jax.lax.broadcasted_iota(jnp.int32, (128, 128), 0)
    c = jax.lax.broadcasted_iota(jnp.int32, (128, 128), 1)
    if inverse:
        r, c = c, r
    src = (c >> 1) + 64 * (c & 1)
    return jnp.where(r == src, 1.0, 0.0).astype(bf16)


def _permute_cols(x, pm):
    parts = [_dot(x[:, j * 128:(j + 1) * 128], pm) for j in range(x.shape[1] // 128)]
    return jnp.concatenate(parts, axis=1)


def _sigmoid(x):
    return 1.0 / (1.0 + jnp.exp(-x))


def _wide(m):
    return jnp.concatenate([m] * NQ, axis=1)


def _fold(a):
    r = a[:, 0:128]
    for j in range(1, NQ):
        r = r + a[:, j * 128:(j + 1) * 128]
    return r


def _rows_loop(n_rows, chunk, fn):
    assert n_rows % chunk == 0

    def body(i, carry):
        fn(pl.ds(pl.multiple_of(i * chunk, chunk), chunk))
        return carry

    jax.lax.fori_loop(0, n_rows // chunk, body, 0)


def _zero(ref, chunk):
    def fn(r):
        ref[r, :] = jnp.zeros((chunk, ref.shape[1]), ref.dtype)
    _rows_loop(ref.shape[0], chunk, fn)


def _cast_to(dst, src, chunk):
    def fn(r):
        dst[r, :] = src[r, :].astype(dst.dtype)
    _rows_loop(src.shape[0], chunk, fn)


def _transpose_to(dst, src):
    def body(i, carry):
        cs = pl.ds(pl.multiple_of(i * 128, 128), 128)
        dst[cs, :] = src[:, cs].T
        return carry
    jax.lax.fori_loop(0, src.shape[1] // 128, body, 0)


def _kernel(x_hbm, wq_hbm, wkT_ref, wvT_ref, wo_hbm, w1T_hbm, w2_hbm, c_ref, wmod_hbm, g_hbm,
            out_hbm, dx_hbm, dwq_hbm, dwkT_ref, dwvT_ref, dwo_hbm, dw1T_hbm, dw2_hbm, dc_ref, dwmod_hbm,
            x_ref, g_ref, wq_ref, wo_ref, w1T, w2_ref, wmod_ref,
            modc, wqT, woT, w1_ref, w2T, wkv, wkvT, xT, st, h1T, qTp, kT, vT1, kN, vN1,
            s_scr, p_scr, m_scr, mp_scr, oT, linv, dh1q, w_scr, dqT,
            dkT, dvT, dxT, dwq_a, dwo_a, dw1_a, dw2_a, dmod_a, dsc_s, row_s, scc_s, dqb_s, dwkv_a, kTf, vTf,
            sem_x, sem_in, sem_out, sem_dx, sem_w):
    MA = 2 * D

    def rows_of(b):
        return pl.ds(pl.multiple_of(b * TQ, TQ), TQ)

    def cp_x(b):
        return pltpu.make_async_copy(x_hbm.at[rows_of(b)], x_ref.at[rows_of(b)], sem_x.at[b])

    def cp_out(b):
        return pltpu.make_async_copy(x_ref.at[rows_of(b)], out_hbm.at[rows_of(b)], sem_out.at[b])

    def cp_dx(b):
        return pltpu.make_async_copy(g_ref.at[rows_of(b)], dx_hbm.at[rows_of(b)], sem_dx.at[b])

    cp_wma = pltpu.make_async_copy(wmod_hbm.at[:, 0:MA], wmod_ref.at[:, 0:MA], sem_in.at[0])
    cp_wq = pltpu.make_async_copy(wq_hbm, wq_ref, sem_in.at[1])
    cp_wmb = pltpu.make_async_copy(wmod_hbm.at[:, MA:6 * D], wmod_ref.at[:, MA:6 * D], sem_in.at[2])
    cp_wo = pltpu.make_async_copy(wo_hbm, wo_ref, sem_in.at[3])
    cp_w1 = pltpu.make_async_copy(w1T_hbm, w1T, sem_in.at[4])
    cp_w2 = pltpu.make_async_copy(w2_hbm, w2_ref, sem_in.at[5])
    cp_g = pltpu.make_async_copy(g_hbm, g_ref, sem_in.at[6])
    co_wq = pltpu.make_async_copy(wq_ref, dwq_hbm, sem_w.at[0])
    co_wo = pltpu.make_async_copy(wo_ref, dwo_hbm, sem_w.at[1])
    co_w1 = pltpu.make_async_copy(w1T, dw1T_hbm, sem_w.at[2])
    co_w2 = pltpu.make_async_copy(w2_ref, dw2_hbm, sem_w.at[3])
    co_wma = pltpu.make_async_copy(wmod_ref.at[:, 0:MA], dwmod_hbm.at[:, 0:MA], sem_w.at[4])
    co_wmb = pltpu.make_async_copy(wmod_ref.at[:, MA:6 * D], dwmod_hbm.at[:, MA:6 * D], sem_w.at[5])

    cp_wma.start()
    cp_x(0).start()
    cp_wq.start()

    c = c_ref[...].astype(f32)
    sig_c = _sigmoid(c)
    sc = c * sig_c
    sc16 = jnp.broadcast_to(sc, (16, D)).astype(bf16)

    wkvT[...] = jnp.zeros((128, D), bf16)
    wkvT[0:DH, :] = wkT_ref[...]
    wkvT[32:32 + DH, :] = wvT_ref[...]
    wkv[...] = wkvT[...].T

    dkT[...] = jnp.zeros_like(dkT)
    dvT[...] = jnp.zeros_like(dvT)
    _zero(dwq_a, 64)
    _zero(dwo_a, 64)
    _zero(dw1_a, 64)
    _zero(dw2_a, 64)
    for j in range(6):
        dmod_a[j] = jnp.zeros((D, 128), f32)
    st[...] = jnp.zeros_like(st)
    dqT[...] = jnp.zeros_like(dqT)

    def set_modc(js):
        mod = _dot(sc16, wmod_ref[:, js[0] * D:(js[-1] + 1) * D])
        for j in js:
            jj = j - js[0]
            mj = jnp.broadcast_to(mod[0:1, jj * D:(jj + 1) * D], (128, D))
            if j in (1, 4):
                mj = mj + 1.0
            modc[j] = mj.T

    cp_wma.wait()
    for b in range(1, NB):
        cp_x(b).start()
    set_modc([0, 1])
    cp_wq.wait()
    _transpose_to(wqT, wq_ref)

    row32 = jax.lax.broadcasted_iota(jnp.int32, (32, TQ), 0)

    def ln_blk(b):
        cols = pl.ds(pl.multiple_of(b * TQ, TQ), TQ)
        xT[:, cols] = x_ref[cols, :].T
        RC = 64
        acc = None
        for r in range(0, D, RC):
            blk = xT[r:r + RC, cols].astype(f32)
            part = jnp.sum(blk.reshape(RC // 8, 8, TQ), axis=0)
            acc = part if acc is None else acc + part
        mu = jnp.sum(acc, axis=0, keepdims=True) * (1.0 / D)
        acc = None
        for r in range(0, D, RC):
            blk = xT[r:r + RC, cols].astype(f32) - mu
            part = jnp.sum((blk * blk).reshape(RC // 8, 8, TQ), axis=0)
            acc = part if acc is None else acc + part
        var = jnp.sum(acc, axis=0, keepdims=True) * (1.0 / D)
        rstd = jax.lax.rsqrt(var + EPS)
        st[0:1, cols] = mu
        st[1:2, cols] = rstd
        for r in range(0, D, RC):
            blk = (xT[r:r + RC, cols].astype(f32) - mu) * rstd
            h1 = blk * _wide(modc[1, r:r + RC, :]) + _wide(modc[0, r:r + RC, :])
            h1T[r:r + RC, cols] = h1.astype(bf16)

    def proj_blk(b):
        cols = pl.ds(pl.multiple_of(b * TQ, TQ), TQ)
        h1b = h1T[:, cols]
        kv = _dot(wkvT[0:64, :], h1b)
        k_t = kv[0:32, :]
        v_t = kv[32:64, :]
        kTf[:, cols] = k_t.astype(bf16).astype(f32)[0:MR]
        v1 = jnp.where(row32 == DH, 1.0, v_t).astype(bf16)
        vTf[:, cols] = _permute_cols(v1, _perm_matrix(False))[0:MR]
        z96 = jnp.zeros((96, TQ), f32)
        hc = pl.ds(pl.multiple_of(b * (TQ // 2), TQ // 2), TQ // 2)
        kN[hc, :] = pltpu.bitcast(jnp.concatenate([k_t, z96], axis=0).T.astype(bf16), u32)
        v11 = jnp.where((row32 == DH) | (row32 == DH + 1), 1.0, v_t)
        vN1[hc, :] = pltpu.bitcast(jnp.concatenate([v11, z96], axis=0).T.astype(bf16), u32)
        QC = 8
        for qc in range(H // QC):
            q = _dot(wqT[qc * QC * DH:(qc + 1) * QC * DH, :], h1b) * (SCALE * LOG2E)
            qz = jnp.concatenate([q, jnp.zeros((16, TQ), f32)], axis=0)
            for h in range(QC):
                qh = jnp.where(row32 < DH, qz[DH * h:DH * h + 32, :], 0.0)
                qTp[qc * QC + h, :, cols] = qh.astype(bf16)

    cp_x(0).wait()
    ln_blk(0)

    def pro_blk(b, carry):
        @pl.when(b + 1 < NB)
        def _():
            cp_x(b + 1).wait()

        @pl.when(b == 1)
        def _():
            cp_wo.start()
            cp_w1.start()
            cp_w2.start()
        proj_blk(b)
        ln_blk(jnp.minimum(b + 1, NB - 1))
        return carry

    jax.lax.fori_loop(0, NB, pro_blk, 0)

    cp_wmb.start()
    cp_g.start()
    cp_wo.wait()
    cp_w1.wait()
    cp_w2.wait()

    def tr_body(i, carry):
        cs = pl.ds(pl.multiple_of(i * 128, 128), 128)
        woT[cs, :] = wo_ref[:, cs].T
        w1_ref[cs, :] = w1T[:, cs].T
        w2T[cs, :] = w2_ref[:, cs].T
        return carry

    jax.lax.fori_loop(0, D // 128, tr_body, 0)

    def stage_a(qt, slot, cc, mx):
        for kk in range(KT):
            r0 = cc * CH + kk * 128
            kblk = pltpu.bitcast(kN[r0 // 2:r0 // 2 + 64, :], bf16)[:, 0:32]
            for qq in range(NQ):
                s = _dot(kblk, qt[:, qq * 128:(qq + 1) * 128])
                s_scr[slot, r0:r0 + 128, qq * 128:(qq + 1) * 128] = s
                sm = jnp.max(s.reshape(16, 8, 128), axis=0)
                mx[qq] = sm if mx[qq] is None else jnp.maximum(mx[qq], sm)

    def finish_max(slot, mx):
        for qq in range(NQ):
            m = jnp.max(mx[qq], axis=0, keepdims=True)
            m_scr[slot, :, qq * 128:(qq + 1) * 128] = jnp.broadcast_to(m, (8, 128))

    mx0 = [None] * NQ
    q00 = qTp[0, :, 0:TQ]
    for cc in range(NC):
        stage_a(q00, 0, cc, mx0)
    finish_max(0, mx0)
    mx1 = [None] * NQ
    q01 = qTp[1, :, 0:TQ]
    for cc in range(LEAD):
        stage_a(q01, 1, cc, mx1)
    for qq in range(NQ):
        mp_scr[:, qq * 128:(qq + 1) * 128] = mx1[qq]

    def finish_mod(j0, j1):
        rows = []
        for j in range(j0, j1):
            t = dmod_a[j].T
            rows.append(jnp.sum(t, axis=0, keepdims=True))
        dmod = jnp.concatenate(rows, axis=1)
        n = (j1 - j0) * D
        hi = dmod.astype(bf16).astype(f32)
        lo = dmod - hi
        r16 = jax.lax.broadcasted_iota(jnp.int32, (16, n), 0)
        dm16 = jnp.where(r16 == 0, hi, jnp.where(r16 == 1, lo, 0.0)).astype(bf16)
        dsc = _dot_nt(dm16, wmod_ref[:, j0 * D:j1 * D])
        row_s[0:1, j0 * D:j1 * D] = dmod
        scc_s[...] = jnp.broadcast_to(sc, (128, D)).T

        def body(i, carry):
            cs = pl.ds(pl.multiple_of(j0 * D + i * 128, 128), 128)
            wmod_ref[:, cs] = (scc_s[...] * row_s[0:1, cs]).astype(bf16)
            return carry

        jax.lax.fori_loop(0, n // 128, body, 0)
        return dsc

    def qproj_bwd(b, hh):
        lc = pl.ds(pl.multiple_of(hh * 128, 128), 128)
        cols = pl.ds(pl.multiple_of(b * TQ + hh * 128, 128), 128)
        dqb = (dqT[:, lc] * SCALE).astype(bf16)
        dwq_a[...] += _dot_nt(h1T[:, cols], dqb)
        dh1q[:, cols] = _dot(wq_ref[...], dqb)

    def block(b, carry):
        cols = pl.ds(pl.multiple_of(b * TQ, TQ), TQ)
        bnext = jnp.minimum(b + 1, NB - 1)

        def fwd_iter(i, carry):
            h0 = i * HPF
            T = HPF * NC
            qslab = {}
            for j in range(1, HPF + 2):
                hh = h0 + j
                wrap = hh >= H
                hq = jnp.where(wrap, hh - H, hh)
                bq = jnp.where(wrap, bnext, b)
                qslab[j] = qTp[hq, :, pl.ds(pl.multiple_of(bq * TQ, TQ), TQ)]
            mx = {1: [mp_scr[:, qq * 128:(qq + 1) * 128] for qq in range(NQ)]}
            for j in range(2, HPF + 2):
                mx[j] = [None] * NQ
            pvals = {}
            acc = {}
            outs = {}

            def stage_b(t):
                j, cc = divmod(t, NC)
                slot = j % 2
                vals = {}
                for kk in range(KT):
                    r0 = cc * CH + kk * 128
                    for qq in range(NQ):
                        m = m_scr[slot, 0:1, qq * 128:(qq + 1) * 128]
                        e = jnp.exp2(s_scr[slot, r0:r0 + 128, qq * 128:(qq + 1) * 128] - m)
                        pk = _pack_halves(e)
                        p_scr[h0 + j, qq, r0 // 2:r0 // 2 + 64, :] = pk
                        vals[(kk, qq)] = pltpu.bitcast(pk, bf16)
                pvals[t] = vals

            def stage_c(t):
                j, cc = divmod(t, NC)
                vals = pvals.pop(t)
                for kk in range(KT):
                    r0 = cc * CH + kk * 128
                    vblk = vTf[:, r0:r0 + 128]
                    for qq in range(NQ):
                        r = _dot(vblk, vals[(kk, qq)])
                        acc[(j, qq)] = r if (j, qq) not in acc else acc[(j, qq)] + r
                if cc == NC - 1:
                    a = jnp.concatenate([acc.pop((j, qq)) for qq in range(NQ)], axis=1)
                    li = 1.0 / a[DH:DH + 1, :]
                    linv[pl.ds(h0 + j, 1), :] = li
                    outs[j] = a[0:DH, :] * li
                    if j % 2 == 1:
                        pair = jnp.concatenate([outs[j - 1], outs[j]], axis=0)
                        r = pl.multiple_of((h0 + j - 1) * DH, 8)
                        oT[pl.ds(r, 2 * DH), :] = pair

            for t in range(T + 1):
                if t < T:
                    ta = t + NC + LEAD
                    ja, ca = divmod(ta, NC)
                    stage_a(qslab[ja], ja % 2, ca, mx[ja])
                    if ca == NC - 1:
                        finish_max(ja % 2, mx[ja])
                    stage_b(t)
                if t >= 1:
                    stage_c(t - 1)
            for qq in range(NQ):
                mp_scr[:, qq * 128:(qq + 1) * 128] = mx[HPF + 1][qq]
            return carry

        jax.lax.fori_loop(0, H // HPF, fwd_iter, 0)

        bprev = jnp.maximum(b - 1, 0)

        @pl.when(b == 0)
        def _():
            cp_wmb.wait()
            set_modc([2, 3, 4, 5])
            cp_g.wait()

        def dense_half(hh, carry):
            lc = pl.ds(pl.multiple_of(hh * 128, 128), 128)
            gc = pl.ds(pl.multiple_of(b * TQ + hh * 128, 128), 128)
            ga_w, sb_w, cb_w, gb_w = modc[2], modc[3], modc[4], modc[5]
            o = oT[:, lc]
            ob = o.astype(bf16)
            gT = g_ref[gc, :].T.astype(f32)
            dfb = (gT * gb_w).astype(bf16)
            a = _dot(woT[...], ob)
            dsT = _dot(w2_ref[...], dfb)
            x1 = xT[:, gc].astype(f32) + ga_w * a
            mu2 = jnp.mean(x1, axis=0, keepdims=True)
            xc2 = x1 - mu2
            var2 = jnp.mean(xc2 * xc2, axis=0, keepdims=True)
            rstd2 = jax.lax.rsqrt(var2 + EPS)
            xh2 = xc2 * rstd2
            h2b = (xh2 * cb_w + sb_w).astype(bf16)
            u = _dot(w1T[...], h2b)
            qproj_bwd(bprev, hh)
            sg = _sigmoid(u)
            sb16 = (u * sg).astype(bf16)
            dub = (dsT * (sg * (1.0 + u * (1.0 - sg)))).astype(bf16)
            dh2 = _dot(w1_ref[...], dub)
            f = _dot(w2T[...], sb16)
            dmod_a[3] += dh2
            dmod_a[4] += dh2 * xh2
            dxh2 = dh2 * cb_w
            dx1 = gT + rstd2 * (dxh2 - jnp.mean(dxh2, axis=0, keepdims=True)
                                - xh2 * jnp.mean(dxh2 * xh2, axis=0, keepdims=True))
            dmod_a[2] += dx1 * a
            dab = (dx1 * ga_w).astype(bf16)
            do = _dot(wo_ref[...], dab)
            dw2_a[...] += _dot_nt(sb16, dfb)
            dw1_a[...] += _dot_nt(dub, h2b)
            dwo_a[...] += _dot_nt(ob, dab)
            outT = x1 + gb_w * f
            x_ref[gc, :] = outT.astype(bf16).T
            dmod_a[5] += gT * f
            dxT[:, gc] = dx1
            for h in range(H):
                li = linv[h:h + 1, lc]
                wr = (do[h * DH:(h + 1) * DH, :] * li).astype(bf16).astype(f32)
                nd = -jnp.sum(wr * o[h * DH:(h + 1) * DH, :], axis=0, keepdims=True)
                hi = nd.astype(bf16).astype(f32)
                lo = nd - hi
                w = jnp.concatenate([wr, hi, lo, jnp.zeros((10, 128), f32)], axis=0)
                w_scr[h, :, lc] = w.astype(bf16)
            return carry

        jax.lax.fori_loop(0, NQ, dense_half, 0)
        cp_out(b).start()

        @pl.when(b == NB - 1)
        def _():
            _cast_to(wo_ref, dwo_a, 64)
            co_wo.start()
            _cast_to(w1T, dw1_a, 64)
            co_w1.start()
            _cast_to(w2_ref, dw2_a, 64)
            co_w2.start()

        def bwd_iter(i, carry):
            h0 = i * HPB
            T = HPB * NC
            ws = {j: w_scr[h0 + j] for j in range(HPB)}
            wf = {j: ws[j].astype(f32)[0:MR] for j in range(HPB)}
            qs = {j: qTp[h0 + j, :, cols].astype(f32)[0:MR] for j in range(HPB)}
            dsv = {}
            dqs = {}
            outs = {}

            def stage1(t):
                j, cc = divmod(t, NC)
                vals = {}
                for kk in range(KT):
                    r0 = cc * CH + kk * 128
                    vblk = pltpu.bitcast(vN1[r0 // 2:r0 // 2 + 64, :], bf16)[:, 0:32]
                    for qq in range(NQ):
                        dp = _dot(vblk, ws[j][:, qq * 128:(qq + 1) * 128])
                        pk = p_scr[h0 + j, qq, r0 // 2:r0 // 2 + 64, :]
                        pf = jnp.concatenate([_unpack_half(pk, 0), _unpack_half(pk, 1)], axis=0)
                        vals[(kk, qq)] = (pf * dp).astype(bf16)
                dsv[t] = vals

            def stage2(t):
                j, cc = divmod(t, NC)
                ds = dsv.pop(t)
                for kk in range(KT):
                    r0 = cc * CH + kk * 128
                    a2 = None
                    for qq in range(NQ):
                        p = pltpu.bitcast(p_scr[h0 + j, qq, r0 // 2:r0 // 2 + 64, :], bf16)
                        r = _dot_nt(wf[j][:, qq * 128:(qq + 1) * 128], p)
                        a2 = r if a2 is None else a2 + r
                    dvT[0:MR, r0:r0 + 128] += a2
                for kk in range(KT):
                    r0 = cc * CH + kk * 128
                    a2 = None
                    for qq in range(NQ):
                        r = _dot_nt(qs[j][:, qq * 128:(qq + 1) * 128], ds[(kk, qq)])
                        a2 = r if a2 is None else a2 + r
                    dkT[0:MR, r0:r0 + 128] += a2
                for kk in range(KT):
                    r0 = cc * CH + kk * 128
                    kblk = kTf[:, r0:r0 + 128]
                    for qq in range(NQ):
                        r = _dot(kblk, ds[(kk, qq)])
                        dqs[(j, qq)] = r if (j, qq) not in dqs else dqs[(j, qq)] + r
                if cc == NC - 1:
                    a3 = jnp.concatenate([dqs.pop((j, qq)) for qq in range(NQ)], axis=1)
                    outs[j] = a3[0:DH, :]
                    if j % 2 == 1:
                        pair = jnp.concatenate([outs[j - 1], outs[j]], axis=0)
                        r = pl.multiple_of((h0 + j - 1) * DH, 8)
                        dqT[pl.ds(r, 2 * DH), :] = pair

            for t in range(T + 1):
                if t < T:
                    stage1(t)
                if t >= 1:
                    stage2(t - 1)
            return carry

        jax.lax.fori_loop(0, H // HPB, bwd_iter, 0)

        return carry

    jax.lax.fori_loop(0, NB, block, 0)

    row32s = jax.lax.broadcasted_iota(jnp.int32, (32, S), 0)
    pinv = _perm_matrix(True)
    kT[...] = jnp.where(row32s < DH, dkT[...] * LN2, 0.0).astype(bf16)
    vT1[...] = _permute_cols(jnp.where(row32s < DH, dvT[...], 0.0).astype(bf16), pinv).astype(bf16)
    dqb_s[...] = (dqT[...] * SCALE).astype(bf16)
    dwkv_a[...] = jnp.zeros_like(dwkv_a)
    dsc_s[...] = finish_mod(2, 6)
    co_wmb.start()
    RQ = D // NB
    last = slice((NB - 1) * TQ, NB * TQ)

    def q_slice(k, live):
        rows = pl.ds(pl.multiple_of(k * RQ, 16), RQ)
        dqb = dqb_s[...]
        dh1q[rows, last] = _dot(wq_ref[rows, :], dqb)
        upd = _dot_nt(h1T[rows, last], dqb)
        dwq_a[rows, :] += upd if live is None else jnp.where(live, upd, 0.0)

    q_slice(0, None)

    def epi_blk(b, carry):
        cols = pl.ds(pl.multiple_of(b * TQ, TQ), TQ)
        dkvb = jnp.concatenate([kT[:, cols], vT1[:, cols]], axis=0)
        dh1 = _dot(wkv[:, 0:64], dkvb) + dh1q[:, cols]
        dwkv_a[...] += _dot_nt(dkvb, h1T[:, cols])
        q_slice(jnp.minimum(b + 1, NB - 1), b + 1 < NB)
        mu = st[0:1, cols]
        rstd = st[1:2, cols]
        xh1 = (xT[:, cols].astype(f32) - mu) * rstd
        dmod_a[0] += _fold(dh1)
        dmod_a[1] += _fold(dh1 * xh1)
        dxh = dh1 * _wide(modc[1])
        dxf = dxT[:, cols] + rstd * (dxh - jnp.mean(dxh, axis=0, keepdims=True)
                                     - xh1 * jnp.mean(dxh * xh1, axis=0, keepdims=True))
        g_ref[cols, :] = dxf.astype(bf16).T
        cp_dx(b).start()
        return carry

    jax.lax.fori_loop(0, NB, epi_blk, 0)
    _cast_to(wq_ref, dwq_a, 64)
    co_wq.start()
    dwkT_ref[...] = dwkv_a[0:DH, :].astype(bf16)
    dwvT_ref[...] = dwkv_a[32:32 + DH, :].astype(bf16)

    dsc = finish_mod(0, 2) + dsc_s[...]
    co_wma.start()
    dsc = dsc[0:1, :] + dsc[1:2, :]
    dc_ref[...] = (dsc * (sig_c * (1.0 + c * (1.0 - sig_c)))).astype(bf16)

    for b in range(NB):
        cp_out(b).wait()
    co_wo.wait()
    co_w1.wait()
    co_w2.wait()
    co_wmb.wait()
    co_wq.wait()
    for b in range(NB):
        cp_dx(b).wait()
    co_wma.wait()


@jax.jit
def pallas_adaLN_cond__grouped_kv_mqa__dense_activation_silu__prompt_kernel(
    A_x: jax.Array,
    A_wq: jax.Array,
    A_wk: jax.Array,
    A_wv: jax.Array,
    A_wo: jax.Array,
    B_x: jax.Array,
    B_w1: jax.Array,
    B_w2: jax.Array,
    c: jax.Array,
    w_mod: jax.Array,
    grad_out: jax.Array,
):
    x = A_x.reshape(S, D)
    g = grad_out.reshape(S, D)
    sds = jax.ShapeDtypeStruct
    out_shape = (
        sds((S, D), bf16), sds((S, D), bf16), sds((D, D), bf16), sds((DH, D), bf16), sds((DH, D), bf16),
        sds((D, D), bf16), sds((F, D), bf16), sds((F, D), bf16), sds((1, D), bf16), sds((D, 6 * D), bf16),
    )
    hbm = pl.BlockSpec(memory_space=pl.ANY)
    vm = pl.BlockSpec(memory_space=pltpu.VMEM)
    in_specs = [hbm, hbm, vm, vm, hbm, hbm, hbm, vm, hbm, hbm]
    out_specs = (hbm, hbm, hbm, vm, vm, hbm, hbm, hbm, vm, hbm)
    V = pltpu.VMEM
    scratch = [
        V((S, D), bf16),
        V((S, D), bf16),
        V((D, D), bf16),
        V((D, D), bf16),
        V((F, D), bf16),
        V((F, D), bf16),
        V((D, 6 * D), bf16),
        V((6, D, 128), f32),
        V((D, D), bf16),
        V((D, D), bf16),
        V((D, F), bf16),
        V((D, F), bf16),
        V((D, 128), bf16),
        V((128, D), bf16),
        V((D, S), bf16),
        V((8, S), f32),
        V((D, S), bf16),
        V((H, 32, S), bf16),
        V((32, S), bf16),
        V((32, S), bf16),
        V((S // 2, 128), u32),
        V((S // 2, 128), u32),
        V((2, S, TQ), f32),
        V((H, NQ, S // 2, 128), u32),
        V((2, 8, TQ), f32),
        V((8, TQ), f32),
        V((D, TQ), f32),
        V((H, TQ), f32),
        V((D, S), f32),
        V((H, 32, TQ), bf16),
        V((D, TQ), f32),
        V((32, S), f32),
        V((32, S), f32),
        V((D, S), f32),
        V((D, D), f32),
        V((D, D), f32),
        V((F, D), f32),
        V((F, D), f32),
        V((6, D, 128), f32),
        V((16, D), f32),
        V((8, 6 * D), f32),
        V((D, 128), f32),
        V((D, TQ), bf16),
        V((64, D), f32),
        V((MR, S), f32),
        V((MR, S), f32),
        pltpu.SemaphoreType.DMA((NB,)),
        pltpu.SemaphoreType.DMA((7,)),
        pltpu.SemaphoreType.DMA((NB,)),
        pltpu.SemaphoreType.DMA((NB,)),
        pltpu.SemaphoreType.DMA((6,)),
    ]
    res = pl.pallas_call(
        _kernel,
        out_shape=out_shape,
        in_specs=in_specs,
        out_specs=out_specs,
        scratch_shapes=scratch,
        compiler_params=pltpu.CompilerParams(vmem_limit_bytes=126 * 1024 * 1024),
    )(x, A_wq, A_wk.T, A_wv.T, A_wo, B_w1.T, B_w2, c, w_mod, g)
    out, dx = res[0].reshape(1, S, D), res[1].reshape(1, S, D)
    return (out, dx, res[2], res[3].T, res[4].T, res[5], res[6].T, res[7], res[8], res[9])
```

```python
import math

import jax
import jax.numpy as jnp
import jax.experimental.pallas as pl
import jax.experimental.pallas.tpu as pltpu

S = 2048
D = 640
H = 32
DH = 20
F = 1728
TQ = 256
NB = S // TQ
NQ = TQ // 128
CH = 256
NC = S // CH
KT = CH // 128
HPF = 8
HPB = 16
LEAD = 2
EPS = 1e-5
SCALE = DH ** -0.5
LOG2E = math.log2(math.e)
LN2 = math.log(2.0)

f32 = jnp.float32
bf16 = jnp.bfloat16
u32 = jnp.uint32
NT = (((1,), (1,)), ((), ()))
NN = (((1,), (0,)), ((), ()))
MR = 24


def _dot(a, b):
    return jax.lax.dot_general(a, b, NN, preferred_element_type=f32)


def _dot_nt(a, b):
    return jax.lax.dot_general(a, b, NT, preferred_element_type=f32)


def _pack2(a, b):
    ua = jax.lax.bitcast_convert_type(a, u32)
    ub = jax.lax.bitcast_convert_type(b, u32)
    return (ua >> 16) | (ub & jnp.uint32(0xFFFF0000))


def _pack_halves(a):
    return _pack2(a[0:64], a[64:128])


def _unpack_half(x, idx):
    y = (x << 16) if idx == 0 else (x & jnp.uint32(0xFFFF0000))
    return jax.lax.bitcast_convert_type(y, f32)


def _perm_matrix(inverse):
    r = jax.lax.broadcasted_iota(jnp.int32, (128, 128), 0)
    c = jax.lax.broadcasted_iota(jnp.int32, (128, 128), 1)
    if inverse:
        r, c = c, r
    src = (c >> 1) + 64 * (c & 1)
    return jnp.where(r == src, 1.0, 0.0).astype(bf16)


def _permute_cols(x, pm):
    parts = [_dot(x[:, j * 128:(j + 1) * 128], pm) for j in range(x.shape[1] // 128)]
    return jnp.concatenate(parts, axis=1)


def _sigmoid(x):
    return 1.0 / (1.0 + jnp.exp(-x))


def _wide(m):
    return jnp.concatenate([m] * NQ, axis=1)


def _fold(a):
    r = a[:, 0:128]
    for j in range(1, NQ):
        r = r + a[:, j * 128:(j + 1) * 128]
    return r


def _rows_loop(n_rows, chunk, fn):
    assert n_rows % chunk == 0

    def body(i, carry):
        fn(pl.ds(pl.multiple_of(i * chunk, chunk), chunk))
        return carry

    jax.lax.fori_loop(0, n_rows // chunk, body, 0)


def _zero(ref, chunk):
    def fn(r):
        ref[r, :] = jnp.zeros((chunk, ref.shape[1]), ref.dtype)
    _rows_loop(ref.shape[0], chunk, fn)


def _cast_to(dst, src, chunk):
    def fn(r):
        dst[r, :] = src[r, :].astype(dst.dtype)
    _rows_loop(src.shape[0], chunk, fn)


def _transpose_to(dst, src):
    def body(i, carry):
        cs = pl.ds(pl.multiple_of(i * 128, 128), 128)
        dst[cs, :] = src[:, cs].T
        return carry
    jax.lax.fori_loop(0, src.shape[1] // 128, body, 0)


def _kernel(x_hbm, wq_hbm, wkT_ref, wvT_ref, wo_hbm, w1T_hbm, w2_hbm, c_ref, wmod_hbm, g_hbm,
            out_hbm, dx_hbm, dwq_hbm, dwkT_ref, dwvT_ref, dwo_hbm, dw1T_hbm, dw2_hbm, dc_ref, dwmod_hbm,
            x_ref, g_ref, wq_ref, wo_ref, w1T, w2_ref, wmod_ref,
            modc, wqT, woT, w1_ref, w2T, wkv, wkvT, xT, st, h1T, qTp, kT, vT1, kN, vN1,
            s_scr, p_scr, m_scr, mp_scr, oT, linv, dh1q, w_scr, dqT,
            dkT, dvT, dxT, dwq_a, dwo_a, dw1_a, dw2_a, dmod_a, dsc_s, row_s, scc_s, dqb_s, dwkv_a, kTf, vTf,
            sem_x, sem_in, sem_out, sem_dx, sem_w):
    MA = 2 * D

    def rows_of(b):
        return pl.ds(pl.multiple_of(b * TQ, TQ), TQ)

    def cp_x(b):
        return pltpu.make_async_copy(x_hbm.at[rows_of(b)], x_ref.at[rows_of(b)], sem_x.at[b])

    def cp_out(b):
        return pltpu.make_async_copy(x_ref.at[rows_of(b)], out_hbm.at[rows_of(b)], sem_out.at[b])

    def cp_dx(b):
        return pltpu.make_async_copy(g_ref.at[rows_of(b)], dx_hbm.at[rows_of(b)], sem_dx.at[b])

    cp_wma = pltpu.make_async_copy(wmod_hbm.at[:, 0:MA], wmod_ref.at[:, 0:MA], sem_in.at[0])
    cp_wq = pltpu.make_async_copy(wq_hbm, wq_ref, sem_in.at[1])
    cp_wmb = pltpu.make_async_copy(wmod_hbm.at[:, MA:6 * D], wmod_ref.at[:, MA:6 * D], sem_in.at[2])
    cp_wo = pltpu.make_async_copy(wo_hbm, wo_ref, sem_in.at[3])
    cp_w1 = pltpu.make_async_copy(w1T_hbm, w1T, sem_in.at[4])
    cp_w2 = pltpu.make_async_copy(w2_hbm, w2_ref, sem_in.at[5])
    cp_g = pltpu.make_async_copy(g_hbm, g_ref, sem_in.at[6])
    co_wq = pltpu.make_async_copy(wq_ref, dwq_hbm, sem_w.at[0])
    co_wo = pltpu.make_async_copy(wo_ref, dwo_hbm, sem_w.at[1])
    co_w1 = pltpu.make_async_copy(w1T, dw1T_hbm, sem_w.at[2])
    co_w2 = pltpu.make_async_copy(w2_ref, dw2_hbm, sem_w.at[3])
    co_wma = pltpu.make_async_copy(wmod_ref.at[:, 0:MA], dwmod_hbm.at[:, 0:MA], sem_w.at[4])
    co_wmb = pltpu.make_async_copy(wmod_ref.at[:, MA:6 * D], dwmod_hbm.at[:, MA:6 * D], sem_w.at[5])

    cp_wma.start()
    cp_x(0).start()
    cp_wq.start()

    c = c_ref[...].astype(f32)
    sig_c = _sigmoid(c)
    sc = c * sig_c
    sc16 = jnp.broadcast_to(sc, (16, D)).astype(bf16)

    wkvT[...] = jnp.zeros((128, D), bf16)
    wkvT[0:DH, :] = wkT_ref[...]
    wkvT[32:32 + DH, :] = wvT_ref[...]
    wkv[...] = wkvT[...].T

    dkT[...] = jnp.zeros_like(dkT)
    dvT[...] = jnp.zeros_like(dvT)
    _zero(dwq_a, 64)
    _zero(dwo_a, 64)
    _zero(dw1_a, 64)
    _zero(dw2_a, 64)
    for j in range(6):
        dmod_a[j] = jnp.zeros((D, 128), f32)
    st[...] = jnp.zeros_like(st)
    dqT[...] = jnp.zeros_like(dqT)

    def set_modc(js):
        mod = _dot(sc16, wmod_ref[:, js[0] * D:(js[-1] + 1) * D])
        for j in js:
            jj = j - js[0]
            mj = jnp.broadcast_to(mod[0:1, jj * D:(jj + 1) * D], (128, D))
            if j in (1, 4):
                mj = mj + 1.0
            modc[j] = mj.T

    cp_wma.wait()
    for b in range(1, NB):
        cp_x(b).start()
    set_modc([0, 1])
    cp_wq.wait()
    _transpose_to(wqT, wq_ref)

    row32 = jax.lax.broadcasted_iota(jnp.int32, (32, TQ), 0)

    def ln_blk(b):
        cols = pl.ds(pl.multiple_of(b * TQ, TQ), TQ)
        xT[:, cols] = x_ref[cols, :].T
        RC = 64
        acc = None
        for r in range(0, D, RC):
            blk = xT[r:r + RC, cols].astype(f32)
            part = jnp.sum(blk.reshape(RC // 8, 8, TQ), axis=0)
            acc = part if acc is None else acc + part
        mu = jnp.sum(acc, axis=0, keepdims=True) * (1.0 / D)
        acc = None
        for r in range(0, D, RC):
            blk = xT[r:r + RC, cols].astype(f32) - mu
            part = jnp.sum((blk * blk).reshape(RC // 8, 8, TQ), axis=0)
            acc = part if acc is None else acc + part
        var = jnp.sum(acc, axis=0, keepdims=True) * (1.0 / D)
        rstd = jax.lax.rsqrt(var + EPS)
        st[0:1, cols] = mu
        st[1:2, cols] = rstd
        for r in range(0, D, RC):
            blk = (xT[r:r + RC, cols].astype(f32) - mu) * rstd
            h1 = blk * _wide(modc[1, r:r + RC, :]) + _wide(modc[0, r:r + RC, :])
            h1T[r:r + RC, cols] = h1.astype(bf16)

    QC = 8

    def q_chunk(qc, h1b, cols):
        q = _dot(wqT[qc * QC * DH:(qc + 1) * QC * DH, :], h1b) * (SCALE * LOG2E)
        qz = jnp.concatenate([q, jnp.zeros((16, TQ), f32)], axis=0)
        for h in range(QC):
            qh = jnp.where(row32 < DH, qz[DH * h:DH * h + 32, :], 0.0)
            qTp[qc * QC + h, :, cols] = qh.astype(bf16)

    def proj_blk(b):
        cols = pl.ds(pl.multiple_of(b * TQ, TQ), TQ)
        h1b = h1T[:, cols]
        kv = _dot(wkvT[0:64, :], h1b)
        k_t = kv[0:32, :]
        v_t = kv[32:64, :]
        kTf[:, cols] = k_t.astype(bf16).astype(f32)[0:MR]
        v1 = jnp.where(row32 == DH, 1.0, v_t).astype(bf16)
        vTf[:, cols] = _permute_cols(v1, _perm_matrix(False))[0:MR]
        z96 = jnp.zeros((96, TQ), f32)
        hc = pl.ds(pl.multiple_of(b * (TQ // 2), TQ // 2), TQ // 2)
        kN[hc, :] = pltpu.bitcast(jnp.concatenate([k_t, z96], axis=0).T.astype(bf16), u32)
        v11 = jnp.where((row32 == DH) | (row32 == DH + 1), 1.0, v_t)
        vN1[hc, :] = pltpu.bitcast(jnp.concatenate([v11, z96], axis=0).T.astype(bf16), u32)
        for qc in range(H // QC - 1):
            q_chunk(qc, h1b, cols)

    cp_x(0).wait()
    ln_blk(0)

    def pro_blk(b, carry):
        @pl.when(b + 1 < NB)
        def _():
            cp_x(b + 1).wait()

        @pl.when(b == 1)
        def _():
            cp_wo.start()
            cp_w1.start()
            cp_w2.start()
        proj_blk(b)
        ln_blk(jnp.minimum(b + 1, NB - 1))
        return carry

    jax.lax.fori_loop(0, NB, pro_blk, 0)

    cp_wmb.start()
    cp_g.start()
    cp_wo.wait()
    cp_w1.wait()
    cp_w2.wait()

    GPI = (NC + LEAD) // (D // 128)
    assert GPI * (D // 128) == NC + LEAD
    BPI = -(-NB // (D // 128))
    m_scr[...] = jnp.full(m_scr.shape, -jnp.inf, f32)

    def tr_body(i, carry):
        cs = pl.ds(pl.multiple_of(i * 128, 128), 128)
        for gi in range(GPI):
            gidx = i * GPI + gi
            hd = gidx // NC
            cc = gidx - hd * NC
            qt = qTp[hd, :, 0:TQ]
            for kk in range(KT):
                r0 = pl.multiple_of(cc * CH + kk * 128, 128)
                rh = pl.multiple_of(cc * (CH // 2) + kk * 64, 64)
                kblk = pltpu.bitcast(kN[pl.ds(rh, 64), :], bf16)[:, 0:32]
                for qq in range(NQ):
                    sv = _dot(kblk, qt[:, qq * 128:(qq + 1) * 128])
                    s_scr[hd, pl.ds(r0, 128), qq * 128:(qq + 1) * 128] = sv
                    sm = jnp.max(sv.reshape(16, 8, 128), axis=0)
                    m_scr[hd, :, qq * 128:(qq + 1) * 128] = jnp.maximum(
                        m_scr[hd, :, qq * 128:(qq + 1) * 128], sm)
        for bi in range(BPI):
            bb = jnp.minimum(i * BPI + bi, NB - 1)
            qcols = pl.ds(pl.multiple_of(bb * TQ, TQ), TQ)
            q_chunk(H // QC - 1, h1T[:, qcols], qcols)
        woT[cs, :] = wo_ref[:, cs].T
        w1_ref[cs, :] = w1T[:, cs].T
        w2T[cs, :] = w2_ref[:, cs].T
        return carry

    jax.lax.fori_loop(0, D // 128, tr_body, 0)

    def stage_a(qt, slot, cc, mx):
        for kk in range(KT):
            r0 = cc * CH + kk * 128
            kblk = pltpu.bitcast(kN[r0 // 2:r0 // 2 + 64, :], bf16)[:, 0:32]
            for qq in range(NQ):
                s = _dot(kblk, qt[:, qq * 128:(qq + 1) * 128])
                s_scr[slot, r0:r0 + 128, qq * 128:(qq + 1) * 128] = s
                sm = jnp.max(s.reshape(16, 8, 128), axis=0)
                mx[qq] = sm if mx[qq] is None else jnp.maximum(mx[qq], sm)

    def finish_max(slot, mx):
        for qq in range(NQ):
            m = jnp.max(mx[qq], axis=0, keepdims=True)
            m_scr[slot, :, qq * 128:(qq + 1) * 128] = jnp.broadcast_to(m, (8, 128))

    mp_scr[...] = m_scr[1]
    finish_max(0, [m_scr[0, :, qq * 128:(qq + 1) * 128] for qq in range(NQ)])

    def finish_mod(j0, j1, mid=None):
        rows = []
        for j in range(j0, j1):
            t = dmod_a[j].T
            rows.append(jnp.sum(t, axis=0, keepdims=True))
        dmod = jnp.concatenate(rows, axis=1)
        n = (j1 - j0) * D
        hi = dmod.astype(bf16).astype(f32)
        lo = dmod - hi
        r16 = jax.lax.broadcasted_iota(jnp.int32, (16, n), 0)
        dm16 = jnp.where(r16 == 0, hi, jnp.where(r16 == 1, lo, 0.0)).astype(bf16)
        dsc = _dot_nt(dm16, wmod_ref[:, j0 * D:j1 * D])
        dsc_s[...] = dsc if j0 > 0 else dsc + dsc_s[...]
        row_s[0:1, j0 * D:j1 * D] = dmod
        scc_s[...] = jnp.broadcast_to(sc, (128, D)).T

        def body(i, carry):
            cs = pl.ds(pl.multiple_of(j0 * D + i * 256, 256), 256)
            wmod_ref[:, cs] = (_wide(scc_s[...]) * row_s[0:1, cs]).astype(bf16)
            return carry

        if mid is not None:
            mid()
        jax.lax.fori_loop(0, n // 256, body, 0)

    def qproj_bwd(b, hh):
        lc = pl.ds(pl.multiple_of(hh * 128, 128), 128)
        cols = pl.ds(pl.multiple_of(b * TQ + hh * 128, 128), 128)
        dqb = (dqT[:, lc] * SCALE).astype(bf16)
        dwq_a[...] += _dot_nt(h1T[:, cols], dqb)
        dh1q[:, cols] = _dot(wq_ref[...], dqb)

    def block(b, carry):
        cols = pl.ds(pl.multiple_of(b * TQ, TQ), TQ)
        bnext = jnp.minimum(b + 1, NB - 1)

        def fwd_iter(i, carry):
            h0 = i * HPF
            T = HPF * NC
            qslab = {}
            for j in range(1, HPF + 2):
                hh = h0 + j
                wrap = hh >= H
                hq = jnp.where(wrap, hh - H, hh)
                bq = jnp.where(wrap, bnext, b)
                qslab[j] = qTp[hq, :, pl.ds(pl.multiple_of(bq * TQ, TQ), TQ)]
            mx = {1: [mp_scr[:, qq * 128:(qq + 1) * 128] for qq in range(NQ)]}
            for j in range(2, HPF + 2):
                mx[j] = [None] * NQ
            pvals = {}
            acc = {}
            outs = {}

            def stage_b(t):
                j, cc = divmod(t, NC)
                slot = j % 2
                vals = {}
                for kk in range(KT):
                    r0 = cc * CH + kk * 128
                    for qq in range(NQ):
                        m = m_scr[slot, 0:1, qq * 128:(qq + 1) * 128]
                        e = jnp.exp2(s_scr[slot, r0:r0 + 128, qq * 128:(qq + 1) * 128] - m)
                        pk = _pack_halves(e)
                        p_scr[h0 + j, qq, r0 // 2:r0 // 2 + 64, :] = pk
                        vals[(kk, qq)] = pltpu.bitcast(pk, bf16)
                pvals[t] = vals

            def stage_c(t):
                j, cc = divmod(t, NC)
                vals = pvals.pop(t)
                for kk in range(KT):
                    r0 = cc * CH + kk * 128
                    vblk = vTf[:, r0:r0 + 128]
                    for qq in range(NQ):
                        r = _dot(vblk, vals[(kk, qq)])
                        acc[(j, qq)] = r if (j, qq) not in acc else acc[(j, qq)] + r
                if cc == NC - 1:
                    a = jnp.concatenate([acc.pop((j, qq)) for qq in range(NQ)], axis=1)
                    li = 1.0 / a[DH:DH + 1, :]
                    linv[pl.ds(h0 + j, 1), :] = li
                    outs[j] = a[0:DH, :] * li
                    if j % 2 == 1:
                        pair = jnp.concatenate([outs[j - 1], outs[j]], axis=0)
                        r = pl.multiple_of((h0 + j - 1) * DH, 8)
                        oT[pl.ds(r, 2 * DH), :] = pair

            for t in range(T + 1):
                if t < T:
                    ta = t + NC + LEAD
                    ja, ca = divmod(ta, NC)
                    stage_a(qslab[ja], ja % 2, ca, mx[ja])
                    if ca == NC - 1:
                        finish_max(ja % 2, mx[ja])
                    stage_b(t)
                if t >= 1:
                    stage_c(t - 1)
            for qq in range(NQ):
                mp_scr[:, qq * 128:(qq + 1) * 128] = mx[HPF + 1][qq]
            return carry

        jax.lax.fori_loop(0, H // HPF, fwd_iter, 0)

        bprev = jnp.maximum(b - 1, 0)

        @pl.when(b == 0)
        def _():
            cp_wmb.wait()
            set_modc([2, 3, 4, 5])
            cp_g.wait()

        def dense_half(hh, carry):
            lc = pl.ds(pl.multiple_of(hh * 128, 128), 128)
            gc = pl.ds(pl.multiple_of(b * TQ + hh * 128, 128), 128)
            ga_w, sb_w, cb_w, gb_w = modc[2], modc[3], modc[4], modc[5]
            o = oT[:, lc]
            ob = o.astype(bf16)
            gT = g_ref[gc, :].T.astype(f32)
            dfb = (gT * gb_w).astype(bf16)
            a = _dot(woT[...], ob)
            dsT = _dot(w2_ref[...], dfb)
            x1 = xT[:, gc].astype(f32) + ga_w * a
            mu2 = jnp.mean(x1, axis=0, keepdims=True)
            xc2 = x1 - mu2
            var2 = jnp.mean(xc2 * xc2, axis=0, keepdims=True)
            rstd2 = jax.lax.rsqrt(var2 + EPS)
            xh2 = xc2 * rstd2
            h2b = (xh2 * cb_w + sb_w).astype(bf16)
            u = _dot(w1T[...], h2b)
            qproj_bwd(bprev, hh)
            sg = _sigmoid(u)
            sb16 = (u * sg).astype(bf16)
            dub = (dsT * (sg * (1.0 + u * (1.0 - sg)))).astype(bf16)
            dh2 = _dot(w1_ref[...], dub)
            f = _dot(w2T[...], sb16)
            dmod_a[3] += dh2
            dmod_a[4] += dh2 * xh2
            dxh2 = dh2 * cb_w
            dx1 = gT + rstd2 * (dxh2 - jnp.mean(dxh2, axis=0, keepdims=True)
                                - xh2 * jnp.mean(dxh2 * xh2, axis=0, keepdims=True))
            dmod_a[2] += dx1 * a
            dab = (dx1 * ga_w).astype(bf16)
            do = _dot(wo_ref[...], dab)
            dw2_a[...] += _dot_nt(sb16, dfb)
            dw1_a[...] += _dot_nt(dub, h2b)
            dwo_a[...] += _dot_nt(ob, dab)
            outT = x1 + gb_w * f
            x_ref[gc, :] = outT.astype(bf16).T
            dmod_a[5] += gT * f
            dxT[:, gc] = dx1
            for h in range(H):
                li = linv[h:h + 1, lc]
                wr = (do[h * DH:(h + 1) * DH, :] * li).astype(bf16).astype(f32)
                nd = -jnp.sum(wr * o[h * DH:(h + 1) * DH, :], axis=0, keepdims=True)
                hi = nd.astype(bf16).astype(f32)
                lo = nd - hi
                w = jnp.concatenate([wr, hi, lo, jnp.zeros((10, 128), f32)], axis=0)
                w_scr[h, :, lc] = w.astype(bf16)
            return carry

        jax.lax.fori_loop(0, NQ, dense_half, 0)
        cp_out(b).start()

        @pl.when(b == NB - 1)
        def _():
            _cast_to(wo_ref, dwo_a, 64)
            co_wo.start()
            _cast_to(w1T, dw1_a, 64)
            co_w1.start()
            _cast_to(w2_ref, dw2_a, 64)
            co_w2.start()

        def bwd_iter(i, carry):
            h0 = i * HPB
            T = HPB * NC
            ws = {j: w_scr[h0 + j] for j in range(HPB)}
            wf = {j: ws[j].astype(f32)[0:MR] for j in range(HPB)}
            qs = {j: qTp[h0 + j, :, cols].astype(f32)[0:MR] for j in range(HPB)}
            dsv = {}
            dqs = {}
            outs = {}

            def stage1(t):
                j, cc = divmod(t, NC)
                vals = {}
                for kk in range(KT):
                    r0 = cc * CH + kk * 128
                    vblk = pltpu.bitcast(vN1[r0 // 2:r0 // 2 + 64, :], bf16)[:, 0:32]
                    for qq in range(NQ):
                        dp = _dot(vblk, ws[j][:, qq * 128:(qq + 1) * 128])
                        pk = p_scr[h0 + j, qq, r0 // 2:r0 // 2 + 64, :]
                        pf = jnp.concatenate([_unpack_half(pk, 0), _unpack_half(pk, 1)], axis=0)
                        vals[(kk, qq)] = (pf * dp).astype(bf16)
                dsv[t] = vals

            def stage2(t):
                j, cc = divmod(t, NC)
                ds = dsv.pop(t)
                for kk in range(KT):
                    r0 = cc * CH + kk * 128
                    a2 = None
                    for qq in range(NQ):
                        p = pltpu.bitcast(p_scr[h0 + j, qq, r0 // 2:r0 // 2 + 64, :], bf16)
                        r = _dot_nt(wf[j][:, qq * 128:(qq + 1) * 128], p)
                        a2 = r if a2 is None else a2 + r
                    dvT[0:MR, r0:r0 + 128] += a2
                for kk in range(KT):
                    r0 = cc * CH + kk * 128
                    a2 = None
                    for qq in range(NQ):
                        r = _dot_nt(qs[j][:, qq * 128:(qq + 1) * 128], ds[(kk, qq)])
                        a2 = r if a2 is None else a2 + r
                    dkT[0:MR, r0:r0 + 128] += a2
                for kk in range(KT):
                    r0 = cc * CH + kk * 128
                    kblk = kTf[:, r0:r0 + 128]
                    for qq in range(NQ):
                        r = _dot(kblk, ds[(kk, qq)])
                        dqs[(j, qq)] = r if (j, qq) not in dqs else dqs[(j, qq)] + r
                if cc == NC - 1:
                    a3 = jnp.concatenate([dqs.pop((j, qq)) for qq in range(NQ)], axis=1)
                    outs[j] = a3[0:DH, :]
                    if j % 2 == 1:
                        pair = jnp.concatenate([outs[j - 1], outs[j]], axis=0)
                        r = pl.multiple_of((h0 + j - 1) * DH, 8)
                        dqT[pl.ds(r, 2 * DH), :] = pair

            for t in range(T + 1):
                if t < T:
                    stage1(t)
                if t >= 1:
                    stage2(t - 1)
            return carry

        jax.lax.fori_loop(0, H // HPB, bwd_iter, 0)

        return carry

    jax.lax.fori_loop(0, NB, block, 0)

    row32s = jax.lax.broadcasted_iota(jnp.int32, (32, S), 0)
    pinv = _perm_matrix(True)
    kT[...] = jnp.where(row32s < DH, dkT[...] * LN2, 0.0).astype(bf16)
    vT1[...] = _permute_cols(jnp.where(row32s < DH, dvT[...], 0.0).astype(bf16), pinv).astype(bf16)
    dqb_s[...] = (dqT[...] * SCALE).astype(bf16)
    dwkv_a[...] = jnp.zeros_like(dwkv_a)
    RQ = D // NB
    last = slice((NB - 1) * TQ, NB * TQ)

    def q_slice(k, live):
        rows = pl.ds(pl.multiple_of(k * RQ, 16), RQ)
        dqb = dqb_s[...]
        dh1q[rows, last] = _dot(wq_ref[rows, :], dqb)
        upd = _dot_nt(h1T[rows, last], dqb)
        dwq_a[rows, :] += upd if live is None else jnp.where(live, upd, 0.0)

    finish_mod(2, 6, lambda: q_slice(0, None))
    co_wmb.start()

    def epi_blk(b, carry):
        cols = pl.ds(pl.multiple_of(b * TQ, TQ), TQ)
        dkvb = jnp.concatenate([kT[:, cols], vT1[:, cols]], axis=0)
        dh1 = _dot(wkv[:, 0:64], dkvb) + dh1q[:, cols]
        dwkv_a[...] += _dot_nt(dkvb, h1T[:, cols])
        q_slice(jnp.minimum(b + 1, NB - 1), b + 1 < NB)
        mu = st[0:1, cols]
        rstd = st[1:2, cols]
        xh1 = (xT[:, cols].astype(f32) - mu) * rstd
        dmod_a[0] += _fold(dh1)
        dmod_a[1] += _fold(dh1 * xh1)
        dxh = dh1 * _wide(modc[1])
        dxf = dxT[:, cols] + rstd * (dxh - jnp.mean(dxh, axis=0, keepdims=True)
                                     - xh1 * jnp.mean(dxh * xh1, axis=0, keepdims=True))
        g_ref[cols, :] = dxf.astype(bf16).T
        cp_dx(b).start()
        return carry

    jax.lax.fori_loop(0, NB, epi_blk, 0)
    _cast_to(wq_ref, dwq_a, 64)
    co_wq.start()
    dwkT_ref[...] = dwkv_a[0:DH, :].astype(bf16)
    dwvT_ref[...] = dwkv_a[32:32 + DH, :].astype(bf16)

    finish_mod(0, 2)
    co_wma.start()
    dsc = dsc_s[0:1, :] + dsc_s[1:2, :]
    dc_ref[...] = (dsc * (sig_c * (1.0 + c * (1.0 - sig_c)))).astype(bf16)

    for b in range(NB):
        cp_out(b).wait()
    co_wo.wait()
    co_w1.wait()
    co_w2.wait()
    co_wmb.wait()
    co_wq.wait()
    for b in range(NB):
        cp_dx(b).wait()
    co_wma.wait()


@jax.jit
def pallas_adaLN_cond__grouped_kv_mqa__dense_activation_silu__prompt_kernel(
    A_x: jax.Array,
    A_wq: jax.Array,
    A_wk: jax.Array,
    A_wv: jax.Array,
    A_wo: jax.Array,
    B_x: jax.Array,
    B_w1: jax.Array,
    B_w2: jax.Array,
    c: jax.Array,
    w_mod: jax.Array,
    grad_out: jax.Array,
):
    x = A_x.reshape(S, D)
    g = grad_out.reshape(S, D)
    sds = jax.ShapeDtypeStruct
    out_shape = (
        sds((S, D), bf16), sds((S, D), bf16), sds((D, D), bf16), sds((DH, D), bf16), sds((DH, D), bf16),
        sds((D, D), bf16), sds((F, D), bf16), sds((F, D), bf16), sds((1, D), bf16), sds((D, 6 * D), bf16),
    )
    hbm = pl.BlockSpec(memory_space=pl.ANY)
    vm = pl.BlockSpec(memory_space=pltpu.VMEM)
    in_specs = [hbm, hbm, vm, vm, hbm, hbm, hbm, vm, hbm, hbm]
    out_specs = (hbm, hbm, hbm, vm, vm, hbm, hbm, hbm, vm, hbm)
    V = pltpu.VMEM
    scratch = [
        V((S, D), bf16),
        V((S, D), bf16),
        V((D, D), bf16),
        V((D, D), bf16),
        V((F, D), bf16),
        V((F, D), bf16),
        V((D, 6 * D), bf16),
        V((6, D, 128), f32),
        V((D, D), bf16),
        V((D, D), bf16),
        V((D, F), bf16),
        V((D, F), bf16),
        V((D, 128), bf16),
        V((128, D), bf16),
        V((D, S), bf16),
        V((8, S), f32),
        V((D, S), bf16),
        V((H, 32, S), bf16),
        V((32, S), bf16),
        V((32, S), bf16),
        V((S // 2, 128), u32),
        V((S // 2, 128), u32),
        V((2, S, TQ), f32),
        V((H, NQ, S // 2, 128), u32),
        V((2, 8, TQ), f32),
        V((8, TQ), f32),
        V((D, TQ), f32),
        V((H, TQ), f32),
        V((D, S), f32),
        V((H, 32, TQ), bf16),
        V((D, TQ), f32),
        V((32, S), f32),
        V((32, S), f32),
        V((D, S), f32),
        V((D, D), f32),
        V((D, D), f32),
        V((F, D), f32),
        V((F, D), f32),
        V((6, D, 128), f32),
        V((16, D), f32),
        V((8, 6 * D), f32),
        V((D, 128), f32),
        V((D, TQ), bf16),
        V((64, D), f32),
        V((MR, S), f32),
        V((MR, S), f32),
        pltpu.SemaphoreType.DMA((NB,)),
        pltpu.SemaphoreType.DMA((7,)),
        pltpu.SemaphoreType.DMA((NB,)),
        pltpu.SemaphoreType.DMA((NB,)),
        pltpu.SemaphoreType.DMA((6,)),
    ]
    res = pl.pallas_call(
        _kernel,
        out_shape=out_shape,
        in_specs=in_specs,
        out_specs=out_specs,
        scratch_shapes=scratch,
        compiler_params=pltpu.CompilerParams(vmem_limit_bytes=126 * 1024 * 1024),
    )(x, A_wq, A_wk.T, A_wv.T, A_wo, B_w1.T, B_w2, c, w_mod, g)
    out, dx = res[0].reshape(1, S, D), res[1].reshape(1, S, D)
    return (out, dx, res[2], res[3].T, res[4].T, res[5], res[6].T, res[7], res[8], res[9])
```
